```python
import jax
import jax.numpy as jnp

def _softmax(x, axis=-1):
    return jax.nn.softmax(x, axis=axis)

def _gelu(x):
    return jax.nn.gelu(x, approximate=True)

def _silu(x):
    return jax.nn.silu(x)

def _sigmoid(x):
    return jax.nn.sigmoid(x)

def _layernorm(x, axis=-1, eps=1e-05):
    m = jnp.mean(x, axis=axis, keepdims=True)
    v = jnp.var(x, axis=axis, keepdims=True)
    return (x - m) / jnp.sqrt(v + eps)

def _scatter_add(tgt, idx, src, axis=0):
    return tgt.at[idx].add(src)

def _segment_sum(src, seg, n):
    return jax.ops.segment_sum(src, seg, n)

class _Rng:

    def __init__(self, key):
        self._k = key

    def _next(self):
        self._k, sub = jax.random.split(self._k)
        return sub

    def normal(self, shape):
        return jax.random.normal(self._next(), shape, dtype=jnp.bfloat16)

    def randint(self, lo, hi, shape):
        return jax.random.randint(self._next(), shape, lo, hi, dtype=jnp.int32)

    def uniform(self, shape, lo=0.0, hi=1.0):
        return jax.random.uniform(self._next(), shape, jnp.bfloat16, lo, hi)

    def permutation(self, n):
        return jax.random.permutation(self._next(), n)
kernel_name = 'interleave_layers__memory_aug_recurrent_mem_tr__ssm_conv_h3__prompt'

def setup_inputs():
    _rng = _Rng(jax.random.key(int.from_bytes(__import__("os").urandom(4), "little")))
    _w = lambda a: (lambda t: t.astype(jnp.bfloat16) if jnp.issubdtype(t.dtype, jnp.floating) else t)(jnp.asarray(a))

    def _A_setup():
        B, S, Dm = (1, 2048, 640)
        H, Dh = (32, 128)
        M, seg = (8, 32)
        seg = min(seg, S)
        S = S // seg * seg
        return {'x': _w((lambda *s: _rng.normal(s) * 0.05)(B, S, Dm)), 'mem0': _w((lambda *s: _rng.normal(s) * 0.05)(B, M, Dm)), 'Wq': _w((lambda *s: _rng.normal(s) * 0.05)(Dm, H, Dh) * Dm ** (-0.5)), 'Wk': _w((lambda *s: _rng.normal(s) * 0.05)(Dm, H, Dh) * Dm ** (-0.5)), 'Wv': _w((lambda *s: _rng.normal(s) * 0.05)(Dm, H, Dh) * Dm ** (-0.5)), 'Wo': _w((lambda *s: _rng.normal(s) * 0.05)(H, Dh, Dm) * (H * Dh) ** (-0.5)), 'seg_len': seg}
    _A_in = _A_setup()

    def _B_setup():
        B, S, D = (1, 2048, 640)
        ks = 4
        return {'q': _w((lambda *s: _rng.normal(s) * 0.05)(B, S, D)), 'k': _w((lambda *s: _rng.normal(s) * 0.05)(B, S, D)), 'v': _w((lambda *s: _rng.normal(s) * 0.05)(B, S, D)), 'shift_k': _w((lambda *s: _rng.normal(s) * 0.05)(D, ks) * 0.5), 'ssm_k': _w((lambda *s: _rng.normal(s) * 0.05)(D, S) * (1.0 / S ** 0.5)), 'ssm_D': _w((lambda *s: _rng.normal(s) * 0.05)(D))}
    _B_in = _B_setup()
    return {'A_x': _A_in['x'], 'A_mem0': _A_in['mem0'], 'A_Wq': _A_in['Wq'], 'A_Wk': _A_in['Wk'], 'A_Wv': _A_in['Wv'], 'A_Wo': _A_in['Wo'], 'A_seg_len': _A_in['seg_len'], 'B_q': _B_in['q'], 'B_k': _B_in['k'], 'B_v': _B_in['v'], 'B_shift_k': _B_in['shift_k'], 'B_ssm_k': _B_in['ssm_k'], 'B_ssm_D': _B_in['ssm_D']}

def reference(A_x, A_mem0, A_Wq, A_Wk, A_Wv, A_Wo, A_seg_len, B_q, B_k, B_v, B_shift_k, B_ssm_k, B_ssm_D):

    def _A_ref(x, mem0, Wq, Wk, Wv, Wo, seg_len):
        B, S, Dm = x.shape
        H, Dh = (Wq.shape[1], Wq.shape[2])
        M = mem0.shape[1]
        scale = Dh ** (-0.5)
        n_seg = S // seg_len
        L = M + seg_len
        idx = jnp.arange(L)
        mask = (idx[:, None] < M) | (idx[:, None] >= idx[None, :])
        mem = mem0
        outs = []
        for s in range(n_seg):
            xs = x[:, s * seg_len:(s + 1) * seg_len, :].copy()
            h = jnp.concatenate([mem, xs], axis=1)
            q = jnp.einsum('btd,dhe->bhte', h, Wq)
            k = jnp.einsum('btd,dhe->bhte', h, Wk)
            v = jnp.einsum('btd,dhe->bhte', h, Wv)
            scores = jnp.einsum('bhqe,bhke->bhqk', q, k) * scale
            scores = jnp.where(mask[None, None], scores, -1000000000.0)
            p = _softmax(scores, axis=-1)
            o = jnp.einsum('bhqk,bhke->bhqe', p, v)
            o = jnp.einsum('bhte,hed->btd', o, Wo)
            mem = o[:, :M, :].copy()
            outs.append(o[:, M:, :])
        return jnp.concatenate(outs, axis=1)

    def _B_ref(q, k, v, shift_k, ssm_k, ssm_D):
        B, S, D = q.shape
        ks = shift_k.shape[-1]
        k_pad = jnp.pad(k, ((0, 0), (ks - 1, 0), (0, 0)))
        k_shift = jnp.zeros_like(k)
        for t in range(ks):
            k_shift = k_shift + k_pad[:, t:t + S, :] * shift_k[:, ks - 1 - t][None, None, :]
        kv = k_shift * v
        L = 2 * S
        kv_pad = jnp.pad(kv, ((0, 0), (0, S), (0, 0)))
        kf_pad = jnp.pad(ssm_k, ((0, 0), (0, S)))
        kv_f = (lambda x, axes=(-2, -1): jnp.fft.rfft2(x.astype(jnp.float32), axes=axes))(kv_pad[:, None, :, :], axes=(1, 2))
        kf_f = (lambda x, axes=(-2, -1): jnp.fft.rfft2(x.astype(jnp.float32), axes=axes))(kf_pad[:, None, :], axes=(1, 2))
        kf_f = (lambda x, *d: x.transpose(*d))(kf_f, 1, 2, 0)
        y_f = kv_f * kf_f[None, :, :, :]
        y = (lambda x, s, axes=(-2, -1): jnp.fft.irfft2(x, s=s, axes=axes).astype(jnp.bfloat16))(y_f, (1, L), axes=(1, 2))[:, 0, :S, :]
        y = y + kv * ssm_D[None, None, :]
        return q * y
    x = A_x
    x = x + _A_ref(_layernorm(x, axis=-1), A_mem0, A_Wq, A_Wk, A_Wv, A_Wo, A_seg_len)
    x = x + _B_ref(_layernorm(x, axis=-1), B_k, B_v, B_shift_k, B_ssm_k, B_ssm_D)
    x = x + _A_ref(_layernorm(x, axis=-1), A_mem0, A_Wq, A_Wk, A_Wv, A_Wo, A_seg_len)
    x = x + _B_ref(_layernorm(x, axis=-1), B_k, B_v, B_shift_k, B_ssm_k, B_ssm_D)
    return x
```

```python
import functools
import numpy as np
import jax
import jax.numpy as jnp
from jax import lax
import jax.experimental.pallas as pl
import jax.experimental.pallas.tpu as pltpu

bf16, f32, u32, i32 = jnp.bfloat16, jnp.float32, jnp.uint32, jnp.int32

LANES = 128
BLK = 128
NFFT = 2 * BLK


def _dft_consts():
    f = np.arange(BLK, dtype=np.float64)[:, None] + 0.5
    m = np.arange(BLK, dtype=np.float64)[None, :]
    ang = 2.0 * np.pi * f * m / NFFT
    fwd = np.concatenate([np.cos(ang), -np.sin(ang)], axis=0)
    inv = np.concatenate([np.cos(ang).T, -np.sin(ang).T], axis=1) * (2.0 / NFFT)
    return fwd.astype(np.float32), inv.astype(np.float32)


def _ln(x):
    m = jnp.mean(x, axis=-1, keepdims=True)
    c = x - m
    v = jnp.mean(c * c, axis=-1, keepdims=True)
    return c * lax.rsqrt(v + 1e-5)


def _ld16(ref_u32):
    return pltpu.bitcast(ref_u32, bf16)


def _make_kernel(S, D, H, DH, M, SEG, KS, lags, opt):
    NSEG = S // SEG
    R = 2 * SEG + 2 * M
    CT = D // LANES
    NB = S // BLK
    HP = H // 2
    scale = DH ** -0.5
    nt = (((1,), (1,)), ((), ()))
    L2E = 1.4426950408889634
    norm = opt.get('norm', 'p'); post_at = opt.get('post_at', 0); wo_mode = opt.get('wo', 'one'); qkv_mode = opt.get('qkv', 'sep'); nr = opt.get('nr', 1)

    def kernel(x_hbm, mem0_ref, wq_hbm, wk_hbm, wv_hbm, wo_hbm, k_hbm, v_hbm, shift_ref, ssm_hbm, ssmd_ref,
               fwd_ref, inv_ref, out_hbm,
               x_s, k_s, v_s, ssm_s, stage_s, w_s, wo_s, y_s, kp_s, kv_s, xf_s, gf_s, z_s,
               lhs_s, x2_s, prev_s, o_s, out_s, sems):
        x32, k32, v32, ssm32 = (r.bitcast(u32) for r in (x_hbm, k_hbm, v_hbm, ssm_hbm))
        wo32 = wo_hbm.bitcast(u32)
        out32 = out_hbm.bitcast(u32)
        w32 = [r.bitcast(u32) for r in (wq_hbm, wk_hbm, wv_hbm)]

        def conv_copies(ct):
            cs = pl.ds(ct * LANES, LANES)
            return (
                pltpu.make_async_copy(k32.at[:, cs], k_s.at[ct], sems.at[0, ct]),
                pltpu.make_async_copy(v32.at[:, cs], v_s.at[ct], sems.at[1, ct]),
                pltpu.make_async_copy(ssm32.at[pl.ds(ct * (LANES // 2), LANES // 2), :], ssm_s.at[ct], sems.at[2, ct]),
            )

        x_copy = pltpu.make_async_copy(x32, x_s, sems.at[3, 0])

        def w_copy(m, i):
            return pltpu.make_async_copy(w32[m].at[:, i, :], stage_s.at[m * HP + i], sems.at[4 + m, i])

        def wo_copy(c):
            return pltpu.make_async_copy(wo32.at[:, pl.ds(c * LANES, LANES)], wo_s.at[c], sems.at[3, 1 + c])

        for ct in range(CT):
            for c in conv_copies(ct):
                c.start()
        x_copy.start()
        for m in range(3):
            for i in range(HP):
                w_copy(m, i).start()
        for c in range(CT):
            wo_copy(c).start()

        fwd = fwd_ref[...]
        inv = inv_ref[...]
        shift_t = shift_ref[...].astype(f32)

        sgn_rows = lax.broadcasted_iota(i32, (BLK, LANES), 0)
        sgn = jnp.where((sgn_rows & 1) == 0, 1.0, -1.0).astype(f32)

        kp_s[0:8, :] = jnp.zeros((8, LANES), f32)
        for ct in range(CT):
            for c in conv_copies(ct):
                c.wait()
            cs = slice(ct * LANES, (ct + 1) * LANES)
            taps = [shift_t[j:j + 1, cs] for j in range(KS)]
            dd = ssmd_ref[pl.ds(ct * LANES, LANES)].astype(f32).reshape(1, LANES)

            def short_a(b, c):
                r = pl.ds(pl.multiple_of(b * (BLK // 2), BLK // 2), BLK // 2)
                kf = _ld16(k_s[ct, r, :]).astype(f32)
                kp_s[pl.ds(pl.multiple_of(8 + b * BLK, 8), BLK), :] = kf
                return c
            lax.fori_loop(0, NB, short_a, 0)

            def short_b(b, c):
                base = pl.multiple_of(8 + b * BLK, 8)
                acc = None
                for j in range(KS):
                    t = kp_s[pl.ds(base - j, BLK), :] * taps[j]
                    acc = t if acc is None else acc + t
                r = pl.ds(pl.multiple_of(b * (BLK // 2), BLK // 2), BLK // 2)
                kv = (acc * _ld16(v_s[ct, r, :]).astype(f32)).astype(bf16)
                kv_s[r, :] = pltpu.bitcast(kv, u32)
                xf_s[b] = jnp.dot(fwd, kv, preferred_element_type=f32)
                sk = _ld16(ssm_s[ct, :, pl.ds(pl.multiple_of(b * BLK, BLK), BLK)])
                gf_s[b] = lax.dot_general(fwd, sk, nt, preferred_element_type=f32)
                return c
            lax.fori_loop(0, NB, short_b, 0)

            def gcomb(t, c):
                cc = NB - 1 - t
                kr, ki = gf_s[cc, 0:BLK, :], gf_s[cc, BLK:NFFT, :]
                pr, pi = gf_s[cc - 1, 0:BLK, :], gf_s[cc - 1, BLK:NFFT, :]
                gf_s[cc, 0:BLK, :] = kr - sgn * pi
                gf_s[cc, BLK:NFFT, :] = ki + sgn * pr
                return c
            lax.fori_loop(0, NB - 1, gcomb, 0)

            def mac(g, c):
                re = pl.ds(pl.multiple_of(g * 16, 16), 16)
                im = pl.ds(pl.multiple_of(BLK + g * 16, 16), 16)
                for a in range(NB):
                    zr = zi = None
                    for b in range(a + 1):
                        gr, gi = gf_s[a - b, re, :], gf_s[a - b, im, :]
                        xr, xi = xf_s[b, re, :], xf_s[b, im, :]
                        pr = gr * xr - gi * xi
                        pi = gr * xi + gi * xr
                        zr = pr if zr is None else zr + pr
                        zi = pi if zi is None else zi + pi
                    z_s[a, pl.ds(pl.multiple_of(g * 8, 8), 8), :] = pltpu.bitcast(zr.astype(bf16), u32)
                    z_s[a, pl.ds(pl.multiple_of(BLK // 2 + g * 8, 8), 8), :] = pltpu.bitcast(zi.astype(bf16), u32)
                return c
            lax.fori_loop(0, BLK // 16, mac, 0)

            def inverse(a, c):
                r = pl.ds(pl.multiple_of(a * (BLK // 2), BLK // 2), BLK // 2)
                y = jnp.dot(inv, _ld16(z_s[a]), preferred_element_type=f32)
                y = y + _ld16(kv_s[r, :]).astype(f32) * dd
                y_s[ct, pl.ds(pl.multiple_of(a * BLK, BLK), BLK), :] = y
                return c
            lax.fori_loop(0, NB, inverse, 0)

        lo_mask = jnp.full((64, LANES), 0xFFFF, u32)
        for m in range(3):
            for i in range(HP):
                w_copy(m, i).wait()

            def relayout(i, c):
                for c0 in range(0, D // 2, 64):
                    E = stage_s[m * HP + i, pl.ds(2 * c0, 64, stride=2), :]
                    O = stage_s[m * HP + i, pl.ds(2 * c0 + 1, 64, stride=2), :]
                    w_s[m, 2 * i, pl.ds(c0, 64), :] = (E & lo_mask) | (O << 16)
                    w_s[m, 2 * i + 1, pl.ds(c0, 64), :] = (E >> 16) | (O & ~lo_mask)
                return c
            lax.fori_loop(0, HP, relayout, 0)
        for c in range(CT):
            wo_copy(c).wait()
        x_copy.wait()

        def xrows(seg):
            return pl.ds(pl.multiple_of(seg * (SEG // 2), SEG // 2), SEG // 2)

        def yrows(seg):
            return pl.ds(pl.multiple_of(seg * SEG, SEG), SEG)

        def load_y(seg):
            return jnp.concatenate([y_s[ct, yrows(seg), :] for ct in range(CT)], axis=1)

        mem0 = mem0_ref[...]
        mem0_2 = jnp.concatenate([mem0, mem0], axis=0)
        lhs_s[0:SEG // 2, :] = pltpu.bitcast(_ln(_ld16(x_s[xrows(0), :]).astype(f32)).astype(bf16), u32)
        lhs_s[SEG // 2:SEG, :] = jnp.zeros((SEG // 2, D), u32)
        lhs_s[SEG:SEG + M, :] = pltpu.bitcast(mem0_2, u32)
        x2_s[0:SEG, :] = jnp.zeros((SEG, D), f32)
        prev_s[...] = jnp.zeros((2 * SEG, D), f32)

        ri = lax.broadcasted_iota(i32, (R, LANES), 0)
        ci = lax.broadcasted_iota(i32, (R, LANES), 1)
        lay_r = jnp.where(ri < 2 * SEG, ri // SEG, (ri - 2 * SEG) // M)
        lay_c = jnp.where(ci < 2 * SEG, ci // SEG, (ci - 2 * SEG) // M)
        mask = (lay_r == lay_c) & ((ri >= 2 * SEG) | (ci >= 2 * SEG) | (ri >= ci))
        lim = jnp.where(mask[:, :R], 3.0e38, -1e9 * L2E).astype(f32)

        def post(j):
            prev = prev_s[...]
            sa = jnp.clip(j - 1, 0, NSEG - 1)
            wa = jnp.clip(j - 1, 0, NSEG)
            sb = jnp.clip(j - 3, 0, NSEG - 1)
            x1 = _ld16(x_s[xrows(sa), :]).astype(f32) + prev[0:SEG]
            x2 = x1 + _ln(x1) * load_y(sa)
            x3 = x2_s[yrows(sb), :] + prev[SEG:2 * SEG]
            x4 = x3 + _ln(x3) * load_y(sb)
            out_s[xrows(sb), :] = pltpu.bitcast(x4.astype(bf16), u32)
            x2_s[yrows(wa), :] = x2
            return x2

        def recip(l):
            r = pl.reciprocal(l, approx=True)
            for _ in range(nr):
                r = r * (2.0 - l * r)
            return r

        def step(j, c):
            lhs = _ld16(lhs_s[...])
            side = {}

            def side_work():
                x2 = post(j)
                side['xn2'] = _ln(x2).astype(bf16)
                s1 = jnp.minimum(j + 1, NSEG - 1)
                side['xn1'] = _ln(_ld16(x_s[xrows(s1), :]).astype(f32)).astype(bf16)

            LAG1, LAG2 = lags
            st = {}
            os_ = {}
            for hh in range(H + LAG2):
                if hh == post_at:
                    side_work()
                if hh < H:
                    if qkv_mode == 'sep':
                        q = jnp.dot(lhs, _ld16(w_s[0, hh]), preferred_element_type=f32).astype(bf16)
                        k = jnp.dot(lhs, _ld16(w_s[1, hh]), preferred_element_type=f32).astype(bf16)
                        v = jnp.dot(lhs, _ld16(w_s[2, hh]), preferred_element_type=f32).astype(bf16)
                    else:
                        w = jnp.concatenate([_ld16(w_s[m, hh]) for m in (1, 0, 2)], axis=1)
                        qkv = jnp.dot(lhs, w, preferred_element_type=f32).astype(bf16)
                        k, q, v = qkv[:, 0:DH], qkv[:, DH:2 * DH], qkv[:, 2 * DH:]
                    st[hh] = (q, k, v)
                h = hh - LAG1
                if 0 <= h < H:
                    q, k, v = st[h]
                    s = lax.dot_general(q, k, nt, preferred_element_type=f32)
                    st[h] = (s, v)
                h = hh - LAG2
                if 0 <= h < H:
                    s, v = st.pop(h)
                    s = jnp.minimum(s * (scale * L2E), lim)
                    mx = jnp.max(s, axis=-1, keepdims=True)
                    e = jnp.exp2(s - mx)
                    l = jnp.sum(e, axis=-1, keepdims=True)
                    if norm == 'p':
                        p = (e * recip(l)).astype(bf16)
                        o = jnp.dot(p, v, preferred_element_type=f32)
                    else:
                        o = jnp.dot(e.astype(bf16), v, preferred_element_type=f32) * recip(l)
                    if opt.get('o_ssa', False):
                        os_[h] = o.astype(bf16)
                    else:
                        o_s[:, h * DH:(h + 1) * DH] = pltpu.bitcast(o.astype(bf16), u32)

            if opt.get('o_ssa', False):
                ob = jnp.concatenate([os_[h] for h in range(H)], axis=1)
            else:
                ob = _ld16(o_s[...])
            if wo_mode == 'one':
                out = jnp.dot(ob, jnp.concatenate([_ld16(wo_s[c]) for c in range(CT)], axis=1), preferred_element_type=f32)
            else:
                out = jnp.concatenate(
                    [jnp.dot(ob, _ld16(wo_s[c]), preferred_element_type=f32) for c in range(CT)], axis=1)
            prev_s[...] = out[0:2 * SEG]
            rowi = lax.broadcasted_iota(i32, (2 * M, D), 0)
            newm = jnp.where((j < 2) & (rowi >= M), mem0_2.astype(f32), out[2 * SEG:]).astype(bf16)
            lhs_s[0:SEG // 2, :] = pltpu.bitcast(side['xn1'], u32)
            lhs_s[SEG // 2:SEG, :] = pltpu.bitcast(side['xn2'], u32)
            lhs_s[SEG:SEG + M, :] = pltpu.bitcast(newm, u32)
            return c

        lax.fori_loop(0, NSEG + 2, step, 0)
        post(NSEG + 2)
        oc = pltpu.make_async_copy(out_s, out32, sems.at[3, 7])
        oc.start()
        oc.wait()

    return kernel


def build(S=2048, D=640, H=32, DH=128, M=8, SEG=32, KS=4, lags=(1, 2), flags=None, **opt):
    R = 2 * SEG + 2 * M
    CT = D // LANES
    NB = S // BLK
    HP = H // 2
    hbm = pl.BlockSpec(memory_space=pl.ANY)
    vm = pl.BlockSpec(memory_space=pltpu.VMEM)
    V = pltpu.VMEM
    scratch = [
        V((S // 2, D), u32),
        V((CT, S // 2, LANES), u32),
        V((CT, S // 2, LANES), u32),
        V((CT, LANES // 2, S), u32),
        V((3 * HP, D, LANES), u32),
        V((3, H, D // 2, LANES), u32),
        V((CT, H * DH // 2, LANES), u32),
        V((CT, S, LANES), f32),
        V((S + 8, LANES), f32),
        V((S // 2, LANES), u32),
        V((NB, NFFT, LANES), f32),
        V((NB, NFFT, LANES), f32),
        V((NB, NFFT // 2, LANES), u32),
        V((R // 2, D), u32),
        V((S + SEG, D), f32),
        V((2 * SEG, D), f32),
        V((R // 2, H * DH), u32),
        V((S // 2, D), u32),
        pltpu.SemaphoreType.DMA((7, 16)),
    ]
    return pl.pallas_call(
        _make_kernel(S, D, H, DH, M, SEG, KS, lags, opt),
        out_shape=jax.ShapeDtypeStruct((S, D), bf16),
        in_specs=[hbm, vm, hbm, hbm, hbm, hbm, hbm, hbm, vm, hbm, vm, vm, vm],
        out_specs=hbm,
        scratch_shapes=scratch,
        compiler_params=pltpu.CompilerParams(vmem_limit_bytes=120 * 1024 * 1024, flags=flags),
    )


def _run(A_x, A_mem0, A_Wq, A_Wk, A_Wv, A_Wo, A_seg_len, B_q, B_k, B_v, B_shift_k, B_ssm_k, B_ssm_D):
    kw = dict(norm='o', lags=(2, 4))
    B, S, D = A_x.shape
    H, DH = A_Wq.shape[1:]
    M = A_mem0.shape[1]
    fwd, inv = _dft_consts()
    call = build(S, D, H, DH, M, int(A_seg_len), B_shift_k.shape[1], **kw)
    out = call(A_x.reshape(S, D), A_mem0.reshape(M, D), A_Wq, A_Wk, A_Wv, A_Wo.reshape(H * DH, D),
               B_k.reshape(S, D), B_v.reshape(S, D), B_shift_k.T, B_ssm_k, B_ssm_D,
               fwd.astype(bf16), inv.astype(bf16))
    return out.reshape(B, S, D)


@functools.partial(jax.jit, static_argnames=('A_seg_len',))
def pallas_interleave_layers__memory_aug_recurrent_mem_tr__ssm_conv_h3__prompt_kernel(
    A_x, A_mem0, A_Wq, A_Wk, A_Wv, A_Wo, A_seg_len, B_q, B_k, B_v, B_shift_k, B_ssm_k, B_ssm_D,
):
    return _run(A_x, A_mem0, A_Wq, A_Wk, A_Wv, A_Wo, A_seg_len, B_q, B_k, B_v, B_shift_k, B_ssm_k, B_ssm_D)
```

```python
import functools
import numpy as np
import jax
import jax.numpy as jnp
from jax import lax
import jax.experimental.pallas as pl
import jax.experimental.pallas.tpu as pltpu

bf16, f32, u32, i32 = jnp.bfloat16, jnp.float32, jnp.uint32, jnp.int32

LANES = 128
BLK = 128
NFFT = 2 * BLK
L2E = 1.4426950408889634


def _dft_consts():
    f = np.arange(BLK, dtype=np.float64)[:, None] + 0.5
    m = np.arange(BLK, dtype=np.float64)[None, :]
    ang = 2.0 * np.pi * f * m / NFFT
    fwd = np.concatenate([np.cos(ang), -np.sin(ang)], axis=0)
    inv = np.concatenate([np.cos(ang).T, -np.sin(ang).T], axis=1) * (2.0 / NFFT)
    return fwd.astype(np.float32), inv.astype(np.float32)


def _ln(x):
    m = jnp.mean(x, axis=-1, keepdims=True)
    c = x - m
    v = jnp.mean(c * c, axis=-1, keepdims=True)
    return c * lax.rsqrt(v + 1e-5)


def _as16(words):
    return pltpu.bitcast(words, bf16)


def _make_kernel(S, D, H, DH, M, SEG, KS, lags, opt):
    NSEG = S // SEG
    R = 2 * SEG + 2 * M
    CT = D // LANES
    NB = S // BLK
    HP = H // 2
    RE = SEG + 2 * M
    scale = DH ** -0.5
    nt = (((1,), (1,)), ((), ()))
    norm = opt.get('norm', 'o'); nr = opt.get('nr', 1)
    clag = opt.get('clag', (1, 2))
    GR = opt.get('gr', 16)
    XHEAD = 8

    def kernel(x_hbm, mem0_ref, wq_hbm, wk_hbm, wv_hbm, wo_hbm, k_hbm, v_hbm, shift_ref, ssm_hbm, ssmd_ref,
               fwd_ref, inv_ref, out_hbm,
               x_s, k_s, v_s, ssm_s, stage_s, w_s, wo_s, y_s, kp_s, par_s, xf_s, gf_s, kraw_s,
               lhs_s, x2_s, prev_s, o_s, out_s, acc_s, sems):
        w32 = [r.bitcast(u32) for r in (wq_hbm, wk_hbm, wv_hbm)]

        def kv_copies(part):
            cs = pl.ds(0, LANES) if part == 0 else pl.ds(LANES, D - LANES)
            return (pltpu.make_async_copy(k_hbm.at[:, cs], k_s.at[:, cs], sems.at[0, part]),
                    pltpu.make_async_copy(v_hbm.at[:, cs], v_s.at[:, cs], sems.at[1, part]))

        def ssm_copy(ct):
            return pltpu.make_async_copy(ssm_hbm.at[pl.ds(ct * LANES, LANES), :], ssm_s.at[ct], sems.at[2, ct])

        xh = XHEAD * SEG
        x_copy0 = pltpu.make_async_copy(x_hbm.at[0:xh], x_s.at[0:xh], sems.at[3, 0])
        x_copy1 = pltpu.make_async_copy(x_hbm.at[xh:S], x_s.at[xh:S], sems.at[3, 6])

        def w_copy(m, i):
            return pltpu.make_async_copy(w32[m].at[:, i, :], stage_s.at[m * HP + i], sems.at[4 + m, i])

        wo_copy = pltpu.make_async_copy(wo_hbm, wo_s, sems.at[3, 1])

        for c in kv_copies(0):
            c.start()
        ssm_copy(0).start()
        for c in kv_copies(1):
            c.start()
        for ct in range(1, CT):
            ssm_copy(ct).start()
        x_copy0.start()
        wo_copy.start()
        for i in range(HP):
            for m in range(3):
                w_copy(m, i).start()

        shift_t = shift_ref[...].astype(f32)
        for ct in range(CT):
            cs = slice(ct * LANES, (ct + 1) * LANES)
            par_s[ct, 0:KS, :] = shift_t[:, cs]
            par_s[ct, KS:KS + 1, :] = ssmd_ref[cs].astype(f32).reshape(1, LANES)
        kp_s[0:8, :] = jnp.zeros((8, LANES), f32)

        def conv_tile(ct, carry):
            for part in range(2):
                @pl.when(ct == part)
                def _():
                    for c in kv_copies(part):
                        c.wait()
            ssm_copy(ct).wait()
            cs = pl.ds(pl.multiple_of(ct * LANES, LANES), LANES)
            fwd = fwd_ref[...]
            inv = inv_ref[...]
            sgn_rows = lax.broadcasted_iota(i32, (BLK, LANES), 0)
            sgn = jnp.where((sgn_rows & 1) == 0, 1.0, -1.0).astype(f32)
            taps = [par_s[ct, j:j + 1, :] for j in range(KS)]
            dd = par_s[ct, KS:KS + 1, :]

            def stage1(b):
                r = slice(b * BLK, (b + 1) * BLK)
                kp_s[8 + b * BLK:8 + (b + 1) * BLK, :] = k_s[r, cs].astype(f32)
                acc = None
                for j in range(KS):
                    t = kp_s[8 + b * BLK - j:8 + (b + 1) * BLK - j, :] * taps[j]
                    acc = t if acc is None else acc + t
                kv = (acc * v_s[r, cs].astype(f32)).astype(bf16)
                y_s[ct, r, :] = kv.astype(f32) * dd
                xf_s[b] = jnp.dot(fwd, kv, preferred_element_type=f32)
                kf = lax.dot_general(fwd, ssm_s[ct, :, r], nt, preferred_element_type=f32)
                if b > 0:
                    pr, pi = kraw_s[(b - 1) % 2, 0:BLK, :], kraw_s[(b - 1) % 2, BLK:NFFT, :]
                    gf_s[b, 0:BLK, :] = kf[0:BLK] - sgn * pi
                    gf_s[b, BLK:NFFT, :] = kf[BLK:NFFT] + sgn * pr
                else:
                    gf_s[b] = kf
                if b < NB - 1:
                    kraw_s[b % 2] = kf

            zs = {}

            def stage2(a):
                zre, zim = [], []
                for g in range(BLK // GR):
                    re = slice(g * GR, (g + 1) * GR)
                    im = slice(BLK + g * GR, BLK + (g + 1) * GR)
                    zr = zi = None
                    for b in range(a + 1):
                        gr, gi = gf_s[a - b, re, :], gf_s[a - b, im, :]
                        xr, xi = xf_s[b, re, :], xf_s[b, im, :]
                        if zr is None:
                            zr = gr * xr - gi * xi
                            zi = gr * xi + gi * xr
                        else:
                            zr = zr + gr * xr - gi * xi
                            zi = zi + gr * xi + gi * xr
                    zre.append(zr.astype(bf16))
                    zim.append(zi.astype(bf16))
                zs[a] = jnp.concatenate(zre + zim, axis=0)

            def stage3(a):
                r = slice(a * BLK, (a + 1) * BLK)
                y_s[ct, r, :] = y_s[ct, r, :] + jnp.dot(inv, zs.pop(a), preferred_element_type=f32)

            l1, l2 = clag
            for t in range(NB + l2):
                if t < NB:
                    stage1(t)
                if 0 <= t - l1 < NB:
                    stage2(t - l1)
                if 0 <= t - l2 < NB:
                    stage3(t - l2)
            return carry

        lax.fori_loop(0, CT, conv_tile, 0)

        def relayout_pair(i):
            lo_mask = jnp.full((64, LANES), 0xFFFF, u32)
            for m in range(3):
                w_copy(m, i).wait()
            for m in range(3):
                for c0 in range(0, D // 2, 64):
                    E = stage_s[m * HP + i, pl.ds(2 * c0, 64, stride=2), :]
                    O = stage_s[m * HP + i, pl.ds(2 * c0 + 1, 64, stride=2), :]
                    w_s[m, 2 * i, pl.ds(c0, 64), :] = (E & lo_mask) | (O << 16)
                    w_s[m, 2 * i + 1, pl.ds(c0, 64), :] = (E >> 16) | (O & ~lo_mask)

        wo_copy.wait()
        x_copy0.wait()
        RA = opt.get('ra', 2)

        def first_hook(hh):
            if hh == 0:
                for i in range(RA + 1):
                    relayout_pair(i)
            elif hh % 2 == 0 and hh // 2 + RA < HP:
                relayout_pair(hh // 2 + RA)

        def rows(seg):
            if isinstance(seg, int):
                return pl.ds(seg * SEG, SEG)
            return pl.ds(pl.multiple_of(seg * SEG, SEG), SEG)

        def clip(j, lo, hi):
            return min(max(j, lo), hi) if isinstance(j, int) else jnp.clip(j, lo, hi)

        def load_y(seg):
            return jnp.concatenate([y_s[ct, rows(seg), :] for ct in range(CT)], axis=1)

        def put_lhs(r0, val):
            n = val.shape[0]
            for c in range(CT):
                lhs_s[c, r0:r0 + n, :] = val[:, c * LANES:(c + 1) * LANES]

        mem0 = mem0_ref[...].astype(f32)
        mem0_2 = jnp.concatenate([mem0, mem0], axis=0)
        put_lhs(0, _ln(x_s[rows(0), :].astype(f32)).astype(bf16))
        put_lhs(SEG, jnp.zeros((SEG, D), bf16))
        put_lhs(2 * SEG, mem0_2.astype(bf16))
        x2_s[0:SEG, :] = jnp.zeros((SEG, D), f32)
        prev_s[...] = jnp.zeros((2 * SEG, D), f32)

        def make_lim(mode):
            n = R if mode == 'full' else RE
            ri = lax.broadcasted_iota(i32, (n, n), 0)
            ci = lax.broadcasted_iota(i32, (n, n), 1)
            nt_ = 2 * SEG if mode == 'full' else SEG

            def lay(i):
                if mode == 'full':
                    return jnp.where(i < nt_, i // SEG, (i - nt_) // M)
                live = 0 if mode == 'e1' else 1
                return jnp.where(i < nt_, 0, jnp.where((i - nt_) // M == live, 0, 1))
            mask = (lay(ri) == lay(ci)) & ((ri >= nt_) | (ci >= nt_) | (ri >= ci))
            return jnp.where(mask, 3.0e38, -1e9 * L2E).astype(f32)

        def post(j, do1=True, do2=True):
            xn2 = None
            if do2:
                sb = clip(j - 3, 0, NSEG - 1)
                x3 = x2_s[rows(sb), :] + prev_s[SEG:2 * SEG, :]
                x4 = x3 + _ln(x3) * load_y(sb)
                out_s[rows(sb), :] = x4.astype(bf16)
            if do1:
                sa = clip(j - 1, 0, NSEG - 1)
                wa = clip(j - 1, 0, NSEG)
                x1 = x_s[rows(sa), :].astype(f32) + prev_s[0:SEG, :]
                x2 = x1 + _ln(x1) * load_y(sa)
                x2_s[rows(wa), :] = x2
                xn2 = _ln(x2).astype(bf16)
            return xn2

        def out_copy(seg):
            return pltpu.make_async_copy(out_s.at[rows(seg)], out_hbm.at[rows(seg)], sems.at[3, 7])

        def recip(l):
            r = pl.reciprocal(l, approx=True)
            for _ in range(nr):
                r = r * (2.0 - l * r)
            return r

        lhs32 = lhs_s.bitcast(u32)
        o32 = o_s.bitcast(u32)

        def make_step(mode, hook=None):
            n = R if mode == 'full' else RE

            def step(j, c):
                lim = make_lim(mode)
                if mode == 'full':
                    lhs = jnp.concatenate([_as16(lhs32[cc]) for cc in range(CT)], axis=1)
                else:
                    t0 = 0 if mode == 'e1' else SEG // 2
                    lhs = jnp.concatenate(
                        [_as16(jnp.concatenate([lhs32[cc, t0:t0 + SEG // 2, :], lhs32[cc, SEG:SEG + M, :]], axis=0))
                         for cc in range(CT)], axis=1)
                first = isinstance(j, int) and j == 0
                xn2 = None if first else post(j, do1=True, do2=(mode != 'e1'))
                if mode != 'e2':
                    s1 = clip(j + 1, 0, NSEG - 1)
                    xn1 = _ln(x_s[rows(s1), :].astype(f32)).astype(bf16)

                LAG1, LAG2 = lags
                G = opt.get('G', 2); WD = opt.get('wd', 8)
                if mode != 'full':
                    LAG1, LAG2 = opt.get('elags', lags)
                    G = opt.get('eG', G); WD = opt.get('ewd', WD)
                NG = H // G
                st = {}
                res = {}

                def wo_group(g):
                    ob = jnp.concatenate([_as16(o32[h, 0:n // 2, :]) for h in range(g * G, (g + 1) * G)], axis=1)
                    kr = slice(g * G * DH, (g + 1) * G * DH)
                    for cc in range(CT):
                        t = jnp.dot(ob, wo_s[kr, cc * LANES:(cc + 1) * LANES], preferred_element_type=f32)
                        if g > 0:
                            t = t + acc_s[cc, 0:n, :]
                        if g < NG - 1:
                            acc_s[cc, 0:n, :] = t
                        else:
                            res[cc] = t

                last = H + LAG2 - 1
                when = {g: min((g + 1) * G - 1 + LAG2 + WD, last) for g in range(NG)}
                for hh in range(H + LAG2):
                    if hook is not None:
                        hook(hh)
                    if hh < H:
                        q = jnp.dot(lhs, _as16(w_s[0, hh]), preferred_element_type=f32).astype(bf16)
                        k = jnp.dot(lhs, _as16(w_s[1, hh]), preferred_element_type=f32).astype(bf16)
                        v = jnp.dot(lhs, _as16(w_s[2, hh]), preferred_element_type=f32).astype(bf16)
                        st[hh] = (q, k, v)
                    h = hh - LAG1
                    if 0 <= h < H:
                        q, k, v = st[h]
                        s = lax.dot_general(q, k, nt, preferred_element_type=f32)
                        st[h] = (s, v)
                    h = hh - LAG2
                    if 0 <= h < H:
                        s, v = st.pop(h)
                        s = jnp.minimum(s * (scale * L2E), lim)
                        mx = jnp.max(s, axis=-1, keepdims=True)
                        e = jnp.exp2(s - mx)
                        l = jnp.sum(e, axis=-1, keepdims=True)
                        o = jnp.dot(e.astype(bf16), v, preferred_element_type=f32) * recip(l)
                        o_s[h, 0:n, :] = o.astype(bf16)
                    for g in range(NG):
                        if when[g] == hh:
                            wo_group(g)

                out = jnp.concatenate([res[cc] for cc in range(CT)], axis=1)
                if mode == 'full':
                    prev_s[...] = out[0:2 * SEG]
                    newm = out[2 * SEG:]
                elif mode == 'e1':
                    prev_s[0:SEG, :] = out[0:SEG]
                    rowi = lax.broadcasted_iota(i32, (2 * M, D), 0)
                    newm = jnp.where(rowi >= M, mem0_2, out[SEG:])
                else:
                    prev_s[SEG:2 * SEG, :] = out[0:SEG]
                    newm = out[SEG:]
                if mode != 'e2':
                    put_lhs(0, xn1)
                if not first:
                    put_lhs(SEG, xn2)
                put_lhs(2 * SEG, newm.astype(bf16))
                if mode != 'e1':
                    @pl.when(j >= 3)
                    def _():
                        out_copy(j - 3).start()
                return c
            return step

        make_step('e1', first_hook)(0, 0)
        x_copy1.start()
        make_step('e1')(1, 0)
        x_copy1.wait()
        UN = opt.get('unroll', 1)
        fstep = make_step('full')
        def ustep(i, c):
            for u in range(UN):
                fstep(2 + i * UN + u, c)
            return c
        lax.fori_loop(0, (NSEG - 2) // UN, ustep, 0)
        lax.fori_loop(NSEG, NSEG + 2, make_step('e2'), 0)
        post(NSEG + 2, do1=False)
        out_copy(NSEG - 1).start()
        pltpu.make_async_copy(out_s, out_hbm, sems.at[3, 7]).wait()

    return kernel


def build(S=2048, D=640, H=32, DH=128, M=8, SEG=32, KS=4, lags=(2, 4), flags=None, **opt):
    R = 2 * SEG + 2 * M
    CT = D // LANES
    NB = S // BLK
    HP = H // 2
    hbm = pl.BlockSpec(memory_space=pl.ANY)
    vm = pl.BlockSpec(memory_space=pltpu.VMEM)
    V = pltpu.VMEM
    scratch = [
        V((S, D), bf16),
        V((S, D), bf16),
        V((S, D), bf16),
        V((CT, LANES, S), bf16),
        V((3 * HP, D, LANES), u32),
        V((3, H, D // 2, LANES), u32),
        V((H * DH, D), bf16),
        V((CT, S, LANES), f32),
        V((S + 8, LANES), f32),
        V((CT, 8, LANES), f32),
        V((NB, NFFT, LANES), f32),
        V((NB, NFFT, LANES), f32),
        V((2, NFFT, LANES), f32),
        V((CT, R, LANES), bf16),
        V((S + SEG, D), f32),
        V((2 * SEG, D), f32),
        V((H, R, DH), bf16),
        V((S, D), bf16),
        V((CT, R, LANES), f32),
        pltpu.SemaphoreType.DMA((7, 16)),
    ]
    return pl.pallas_call(
        _make_kernel(S, D, H, DH, M, SEG, KS, lags, opt),
        out_shape=jax.ShapeDtypeStruct((S, D), bf16),
        in_specs=[hbm, vm, hbm, hbm, hbm, hbm, hbm, hbm, vm, hbm, vm, vm, vm],
        out_specs=hbm,
        scratch_shapes=scratch,
        compiler_params=pltpu.CompilerParams(vmem_limit_bytes=120 * 1024 * 1024, flags=flags),
    )


def _run(A_x, A_mem0, A_Wq, A_Wk, A_Wv, A_Wo, A_seg_len, B_q, B_k, B_v, B_shift_k, B_ssm_k, B_ssm_D):
    kw = dict()
    B, S, D = A_x.shape
    H, DH = A_Wq.shape[1:]
    M = A_mem0.shape[1]
    fwd, inv = _dft_consts()
    call = build(S, D, H, DH, M, int(A_seg_len), B_shift_k.shape[1], **kw)
    out = call(A_x.reshape(S, D), A_mem0.reshape(M, D), A_Wq, A_Wk, A_Wv, A_Wo.reshape(H * DH, D),
               B_k.reshape(S, D), B_v.reshape(S, D), B_shift_k.T, B_ssm_k, B_ssm_D,
               fwd.astype(bf16), inv.astype(bf16))
    return out.reshape(B, S, D)


@functools.partial(jax.jit, static_argnames=('A_seg_len',))
def pallas_interleave_layers__memory_aug_recurrent_mem_tr__ssm_conv_h3__prompt_kernel(
    A_x, A_mem0, A_Wq, A_Wk, A_Wv, A_Wo, A_seg_len, B_q, B_k, B_v, B_shift_k, B_ssm_k, B_ssm_D,
):
    return _run(A_x, A_mem0, A_Wq, A_Wk, A_Wv, A_Wo, A_seg_len, B_q, B_k, B_v, B_shift_k, B_ssm_k, B_ssm_D)
```

```python
import functools
import numpy as np
import jax
import jax.numpy as jnp
from jax import lax
import jax.experimental.pallas as pl
import jax.experimental.pallas.tpu as pltpu

bf16, f32, u32, i32 = jnp.bfloat16, jnp.float32, jnp.uint32, jnp.int32

LANES = 128
BLK = 128
NFFT = 2 * BLK
L2E = 1.4426950408889634


def _dft_consts():
    f = np.arange(BLK, dtype=np.float64)[:, None] + 0.5
    m = np.arange(BLK, dtype=np.float64)[None, :]
    ang = 2.0 * np.pi * f * m / NFFT
    fwd = np.concatenate([np.cos(ang), -np.sin(ang)], axis=0)
    inv = np.concatenate([np.cos(ang).T, -np.sin(ang).T], axis=1) * (2.0 / NFFT)
    return fwd.astype(np.float32), inv.astype(np.float32)


def _ln(x):
    m = jnp.mean(x, axis=-1, keepdims=True)
    c = x - m
    v = jnp.mean(c * c, axis=-1, keepdims=True)
    return c * lax.rsqrt(v + 1e-5)


def _as16(words):
    return pltpu.bitcast(words, bf16)


def _plan(S, D, SEG, opt):
    NSEG = S // SEG
    CT = D // LANES
    NB = S // BLK
    NP = opt.get('na', 9)
    EB = opt.get('eb', 4)
    UPS = opt.get('ups', 2)
    assert ((NB - EB) * CT) % UPS == 0
    NU = (NB - EB) * CT // UPS
    assert NP + NU <= NSEG
    return NP, EB, UPS, NU


def _make_kernel(S, D, H, DH, M, SEG, KS, lags, opt):
    NSEG = S // SEG
    R = 2 * SEG + 2 * M
    RE = SEG + 2 * M
    CT = D // LANES
    NB = S // BLK
    HP = H // 2
    scale = DH ** -0.5
    nt = (((1,), (1,)), ((), ()))
    nr = opt.get('nr', 1)
    GR = opt.get('gr', 16)
    NP, EB, UPS, NU = _plan(S, D, SEG, opt)
    XHEAD = (NP + 2) * SEG
    PR = NP * SEG
    ALLPRE = opt.get('allpre', True)
    ZB = H * R
    NXZ = -(-CT * NB // HP)
    NGZ = -(-(CT * (NB + 1) + NB - 1) // HP)
    GP = NB - 1
    XO = opt.get('xo', 16); XS = opt.get('xs', NFFT + 32)

    def kernel(x_hbm, mem0_hbm, wq_hbm, wk_hbm, wv_hbm, wo_hbm, k_hbm, v_hbm, shift_hbm, ssm_hbm, ssmd_hbm,
               fwd_hbm, inv_hbm, out_hbm,
               mem0_ref, shift_ref, ssmd_ref, fwd_ref, inv_ref,
               x_s, k_s, v_s, ssm_s, stage_s, w_s, wo_s, y_s, kq_s, par_s, xg_s, gg_s, kr_s,
               lhs_s, x2_s, prev_s, o_s, out_s, acc_s, xn_s, pre_s, sems):
        w32 = [r.bitcast(u32) for r in (wq_hbm, wk_hbm, wv_hbm)]
        small = [pltpu.make_async_copy(a, b, sems.at[3, 8 + i]) for i, (a, b) in enumerate(
            [(shift_hbm, shift_ref), (ssmd_hbm, ssmd_ref), (fwd_hbm, fwd_ref), (inv_hbm, inv_ref), (mem0_hbm, mem0_ref)])]
        x_copy = [pltpu.make_async_copy(x_hbm.at[a:b], x_s.at[a:b], sems.at[3, i]) for i, (a, b) in enumerate([(0, XHEAD), (XHEAD, S)])]
        E0 = EB * BLK

        def conv_copies(part):
            sl = slice(0, E0) if part == 0 else slice(E0, S)
            return (pltpu.make_async_copy(k_hbm.at[sl], k_s.at[sl], sems.at[0, part]),
                    pltpu.make_async_copy(v_hbm.at[sl], v_s.at[sl], sems.at[1, part]),
                    pltpu.make_async_copy(ssm_hbm.at[:, sl], ssm_s.at[:, sl], sems.at[2, part]))

        def w_copy(m, i):
            return pltpu.make_async_copy(w32[m].at[:, i, :], stage_s.at[m * HP + i], sems.at[4 + m, i])

        wo_copy = pltpu.make_async_copy(wo_hbm, wo_s, sems.at[3, 2])

        for c in small:
            c.start()
        x_copy[0].start()
        for i in range(HP):
            for m in range(3):
                w_copy(m, i).start()
        for c in conv_copies(0):
            c.start()
        wo_copy.start()
        for c in conv_copies(1):
            c.start()
        x_copy[1].start()

        for c in small:
            c.wait()
        x_copy[0].wait()
        for r0 in range(0, PR, SEG):
            r = slice(r0, r0 + SEG)
            xn = _ln(x_s[r, :].astype(f32)).astype(bf16)
            for cc in range(CT):
                xn_s[cc, r, :] = xn[:, cc * LANES:(cc + 1) * LANES]
        if ALLPRE:
            m0 = mem0_ref[...]
            for cc in range(CT):
                xn_s[cc, PR:PR + 2 * M, :] = jnp.concatenate([m0, m0], axis=0)[:, cc * LANES:(cc + 1) * LANES]
        xn32 = xn_s.bitcast(u32)
        lhs32 = lhs_s.bitcast(u32)
        o32 = o_s.bitcast(u32)

        def phase_a(i, carry):
            lo_mask = jnp.full((64, LANES), 0xFFFF, u32)
            for m in range(3):
                pltpu.make_async_copy(stage_s.at[m * HP + i], stage_s.at[m * HP + i], sems.at[4 + m, i]).wait()

            def relayout(m):
                for c0 in range(0, D // 2, 64):
                    E = stage_s[m * HP + i, pl.ds(2 * c0, 64, stride=2), :]
                    O = stage_s[m * HP + i, pl.ds(2 * c0 + 1, 64, stride=2), :]
                    w_s[m, 2 * i, pl.ds(c0, 64), :] = (E & lo_mask) | (O << 16)
                    w_s[m, 2 * i + 1, pl.ds(c0, 64), :] = (E >> 16) | (O & ~lo_mask)

            lhs = jnp.concatenate([_as16(xn32[cc]) for cc in range(CT)], axis=1)
            order = opt.get('aord', 0)
            if order == 0:
                for m in range(3):
                    relayout(m)
            for m in range(3):
                if order == 1:
                    relayout(m)
                for hh in range(2):
                    r = jnp.dot(lhs, _as16(w_s[m, 2 * i + hh]), preferred_element_type=f32)
                    pre_s[m, 2 * i + hh] = r.astype(bf16)
            return carry

        lax.fori_loop(0, HP, phase_a, 0)

        shift_t = shift_ref[...].astype(f32)
        for ct in range(CT):
            cs = slice(ct * LANES, (ct + 1) * LANES)
            par_s[ct, 0:KS, :] = shift_t[:, cs]
            par_s[ct, KS:KS + 1, :] = ssmd_ref[cs].astype(f32).reshape(1, LANES)

        def conv_front(a, ct, slot, kprev=None, keep=True):
            static = isinstance(a, int)
            fwd = fwd_ref[...]
            cs = pl.ds(ct * LANES, LANES) if isinstance(ct, int) else pl.ds(pl.multiple_of(ct * LANES, LANES), LANES)
            r = pl.ds(a * BLK, BLK) if static else pl.ds(pl.multiple_of(a * BLK, BLK), BLK)
            sgn_rows = lax.broadcasted_iota(i32, (BLK, LANES), 0)
            sgn = jnp.where((sgn_rows & 1) == 0, 1.0, -1.0).astype(f32)
            if static and a == 0:
                kq_s[slot, 0:16, :] = jnp.zeros((16, LANES), f32)
                kq_s[slot, 16:, :] = k_s[r, cs].astype(f32)
            elif static:
                kq_s[slot] = k_s[pl.ds(a * BLK - 16, BLK + 16), cs].astype(f32)
            else:
                kq_s[slot] = k_s[pl.ds(pl.multiple_of(a * BLK - 16, 16), BLK + 16), cs].astype(f32)
            acc = None
            for jj in range(KS):
                t = kq_s[slot, 16 - jj:16 - jj + BLK, :] * par_s[ct, jj:jj + 1, :]
                acc = t if acc is None else acc + t
            kv = (acc * v_s[r, cs].astype(f32)).astype(bf16)
            y_s[ct, r, :] = kv.astype(f32) * par_s[ct, KS:KS + 1, :]
            base = ct * NB
            gbase = ct * (NB + 1) + GP
            xg_s[base + a, XO:XO + NFFT, :] = jnp.dot(fwd, kv, preferred_element_type=f32)
            kf = lax.dot_general(fwd, ssm_s[cs, r], nt, preferred_element_type=f32)
            if static and a == 0:
                gg_s[gbase + a] = kf
            else:
                pr, pi = (kr_s[ct, 0:BLK, :], kr_s[ct, BLK:NFFT, :]) if kprev is None else (kprev[0:BLK], kprev[BLK:NFFT])
                gg_s[gbase + a, 0:BLK, :] = kf[0:BLK] - sgn * pi
                gg_s[gbase + a, BLK:NFFT, :] = kf[BLK:NFFT] + sgn * pr
            if keep:
                kr_s[ct] = kf
            return kf

        def conv_mac(a, ct, nout, zero, slot0=0, GR=GR):
            static = isinstance(a, int)
            base = ct * NB
            g0 = ct * (NB + 1) + a
            nb = a + nout if static else NB
            for g in range(BLK // GR):
                re = slice(g * GR, (g + 1) * GR)
                im = slice(BLK + g * GR, BLK + (g + 1) * GR)
                xre = slice(re.start + XO, re.stop + XO)
                xim = slice(im.start + XO, im.stop + XO)
                z = [None] * nout
                gwin = {}
                for b in range(nb):
                    xr, xi = xg_s[base + b, xre, :], xg_s[base + b, xim, :]
                    for o in range(nout):
                        c = o - b
                        if static and a + c < 0:
                            continue
                        if c not in gwin:
                            gwin[c] = (gg_s[g0 + (GP + c), re, :], gg_s[g0 + (GP + c), im, :])
                        gr, gi = gwin[c]
                        if z[o] is None:
                            z[o] = (gr * xr - gi * xi, gr * xi + gi * xr)
                        else:
                            z[o] = (z[o][0] + gr * xr - gi * xi, z[o][1] + gr * xi + gi * xr)
                    gwin.pop(nout - 1 - b, None)
                for o in range(nout):
                    zb = ZB + (slot0 + o) * NFFT + zero
                    mo = (lambda v: v) if isinstance(zb, int) else (lambda v: pl.multiple_of(v, GR))
                    o_s[pl.ds(mo(zb + g * GR), GR), :] = z[o][0].astype(bf16)
                    o_s[pl.ds(mo(zb + BLK + g * GR), GR), :] = z[o][1].astype(bf16)
                yield

        def conv_back(a, ct, o):
            static = isinstance(a, int)
            r = pl.ds(a * BLK, BLK) if static else pl.ds(pl.multiple_of(a * BLK, BLK), BLK)
            z = _as16(o32[(ZB + o * NFFT) // 2:(ZB + (o + 1) * NFFT) // 2, :])
            y_s[ct, r, :] = y_s[ct, r, :] + jnp.dot(inv_ref[...], z, preferred_element_type=f32)

        def conv_unit(a, ct, nout, zero):
            for o in range(nout):
                conv_front(a + o, ct, o)
                yield
            yield from conv_mac(a, ct, nout, zero)
            for o in range(nout):
                conv_back(a + o, ct, o)
            yield

        for c in conv_copies(0):
            c.wait()

        def early_conv(ct, carry):
            zero = 0 if isinstance(ct, int) else jnp.minimum(ct, 0)
            if opt.get('epipe', True):
                l1, l2 = opt.get('eclag', (1, 2))
                kprev = None
                for t in range(EB + l2):
                    if t < EB:
                        kprev = conv_front(t, ct, t % UPS, kprev if opt.get('kssa', True) else None, keep=(t == EB - 1 or not opt.get('kssa', True)))
                    if 0 <= t - l1 < EB:
                        for _ in conv_mac(t - l1, ct, 1, zero, (t - l1) % UPS, opt.get('egr', 16)):
                            pass
                    if 0 <= t - l2 < EB:
                        conv_back(t - l2, ct, (t - l2) % UPS)
            else:
                for _ in conv_unit(0, ct, EB, zero):
                    pass
            return carry

        if opt.get('estatic', True):
            for ct_ in range(CT):
                early_conv(ct_, 0)
        else:
            lax.fori_loop(0, CT, early_conv, 0)

        wo_copy.wait()

        def rows(seg):
            if isinstance(seg, int):
                return pl.ds(seg * SEG, SEG)
            return pl.ds(pl.multiple_of(seg * SEG, SEG), SEG)

        def clip(j, lo, hi):
            return min(max(j, lo), hi) if isinstance(j, int) else jnp.clip(j, lo, hi)

        def load_y(seg):
            return jnp.concatenate([y_s[ct, rows(seg), :] for ct in range(CT)], axis=1)

        def put_lhs(r0, val):
            n = val.shape[0]
            for c in range(CT):
                lhs_s[c, r0:r0 + n, :] = val[:, c * LANES:(c + 1) * LANES]

        mem0 = mem0_ref[...].astype(f32)
        mem0_2 = jnp.concatenate([mem0, mem0], axis=0)
        put_lhs(0, jnp.zeros((2 * SEG, D), bf16))
        put_lhs(2 * SEG, mem0_2.astype(bf16))
        x2_s[0:SEG, :] = jnp.zeros((SEG, D), f32)
        prev_s[...] = jnp.zeros((2 * SEG, D), f32)

        def make_lim(mode):
            n = R if mode == 'full' else RE
            ri = lax.broadcasted_iota(i32, (n, n), 0)
            ci = lax.broadcasted_iota(i32, (n, n), 1)
            nt_ = 2 * SEG if mode == 'full' else SEG

            def lay(i):
                if mode == 'full':
                    return jnp.where(i < nt_, i // SEG, (i - nt_) // M)
                live = 0 if mode == 'e1' else 1
                return jnp.where(i < nt_, 0, jnp.where((i - nt_) // M == live, 0, 1))
            mask = (lay(ri) == lay(ci)) & ((ri >= nt_) | (ci >= nt_) | (ri >= ci))
            return jnp.where(mask, 3.0e38, -1e9 * L2E).astype(f32)

        def post(j, do1=True, do2=True):
            xn2 = None
            if do2:
                sb = clip(j - 3, 0, NSEG - 1)
                x3 = x2_s[rows(sb), :] + prev_s[SEG:2 * SEG, :]
                x4 = x3 + _ln(x3) * load_y(sb)
                out_s[rows(sb), :] = x4.astype(bf16)
            if do1:
                sa = clip(j - 1, 0, NSEG - 1)
                wa = clip(j - 1, 0, NSEG)
                x1 = x_s[rows(sa), :].astype(f32) + prev_s[0:SEG, :]
                x2 = x1 + _ln(x1) * load_y(sa)
                x2_s[rows(wa), :] = x2
                xn2 = _ln(x2).astype(bf16)
            return xn2

        def out_copy(seg):
            return pltpu.make_async_copy(out_s.at[rows(seg)], out_hbm.at[rows(seg)], sems.at[3, 7])

        def recip(l):
            r = pl.reciprocal(l, approx=True)
            for _ in range(nr):
                r = r * (2.0 - l * r)
            return r

        def make_step(mode, pre=False, units=0):
            n = R if mode == 'full' else RE

            def step(j, c):
                lim = make_lim(mode)
                if mode == 'full' and not pre:
                    lhs = jnp.concatenate([_as16(lhs32[cc]) for cc in range(CT)], axis=1)
                elif mode == 'full':
                    lhs = jnp.concatenate([_as16(lhs32[cc, SEG // 2:R // 2, :]) for cc in range(CT)], axis=1)
                elif pre:
                    lhs = jnp.concatenate([_as16(lhs32[cc, SEG:SEG + M, :]) for cc in range(CT)], axis=1)
                else:
                    t0 = 0 if mode == 'e1' else SEG // 2
                    lhs = jnp.concatenate(
                        [_as16(jnp.concatenate([lhs32[cc, t0:t0 + SEG // 2, :], lhs32[cc, SEG:SEG + M, :]], axis=0))
                         for cc in range(CT)], axis=1)

                def proj(m, h):
                    if pre == 'all':
                        return jnp.concatenate([pre_s[m, h, rows(j), :], pre_s[m, h, PR:PR + 2 * M, :]], axis=0)
                    r = jnp.dot(lhs, _as16(w_s[m, h]), preferred_element_type=f32).astype(bf16)
                    if pre:
                        r = jnp.concatenate([pre_s[m, h, rows(j), :], r], axis=0)
                    return r

                sched = {}
                if units:
                    u0, u1 = opt.get('uspan', (8, 35))
                    gap = opt.get('ugap', 2)
                    u = j - NP
                    gen = conv_unit(EB + (u // CT) * units, u % CT, units, jnp.minimum(j, 0))
                    nmac = BLK // GR
                    fs = opt.get('fstep', 1)
                    for o in range(units):
                        sched.setdefault(u0 + o * fs, []).append(gen)
                    m0 = u0 + units * fs + gap
                    for p in range(nmac):
                        hh_ = int(round(m0 + p * (u1 - m0 - 1) / (nmac - 1)))
                        sched.setdefault(hh_, []).append(gen)
                    sched.setdefault(hh_ + 1, []).append(gen)

                zfill = {}
                if mode == 'full' and pre:
                    NZ = NB - EB
                    nx, ng = CT * NZ, GP + CT * (NZ + 1)
                    nsteps = NP - 2
                    px, pg = -(-nx // nsteps), -(-ng // nsteps)
                    zblk = jnp.zeros((NFFT, LANES), f32)
                    items = []
                    for q_ in range(px):
                        kx = jnp.minimum((j - 2) * px + q_, nx - 1)
                        items.append((xg_s, (kx // NZ) * NB + EB + kx % NZ, XO))
                    for q_ in range(pg):
                        kg = jnp.minimum((j - 2) * pg + q_, ng - 1)
                        kk = jnp.maximum(kg - GP, 0)
                        items.append((gg_s, jnp.where(kg < GP, kg, GP + (kk // (NZ + 1)) * (NB + 1) + EB + kk % (NZ + 1)), 0))
                    for q_, it in enumerate(items):
                        zfill.setdefault(q_ * H // len(items), []).append(it)
                first = isinstance(j, int) and j == 0
                xn2 = None if first else post(j, do1=True, do2=(mode != 'e1'))
                need_xn1 = mode == 'full'
                if need_xn1:
                    s1 = clip(j + 1, 0, NSEG - 1)
                    xn1 = _ln(x_s[rows(s1), :].astype(f32)).astype(bf16)

                LAG1, LAG2 = lags
                G = opt.get('G', 2); WD = opt.get('wd', 8)
                if mode != 'full':
                    LAG1, LAG2 = opt.get('elags', lags)
                    if pre == 'all':
                        LAG1, LAG2 = opt.get('alags', (0, 4))
                    G = opt.get('eG', G); WD = opt.get('ewd', WD)
                if units:
                    G = opt.get('uG', G); WD = opt.get('uwd', WD); LAG1, LAG2 = opt.get('ulags', (LAG1, LAG2))
                NG = H // G
                st = {}
                res = {}

                def wo_group(g):
                    ob = jnp.concatenate([_as16(o32[h * R // 2:(h * R + n) // 2, :]) for h in range(g * G, (g + 1) * G)], axis=1)
                    kr = slice(g * G * DH, (g + 1) * G * DH)
                    for cc in range(CT):
                        t = jnp.dot(ob, wo_s[kr, cc * LANES:(cc + 1) * LANES], preferred_element_type=f32)
                        if g > 0:
                            t = t + acc_s[cc, 0:n, :]
                        if g < NG - 1:
                            acc_s[cc, 0:n, :] = t
                        else:
                            res[cc] = t

                last = H + LAG2 - 1
                when = {g: min((g + 1) * G - 1 + LAG2 + WD, last) for g in range(NG)}
                for hh in range(H + LAG2):
                    for gen in sched.get(hh, []):
                        next(gen)
                    for ref, idx, off in zfill.get(hh, []):
                        ref[idx, off:off + NFFT, :] = zblk
                    if hh < H:
                        st[hh] = (proj(0, hh), proj(1, hh), proj(2, hh))
                    h = hh - LAG1
                    if 0 <= h < H:
                        q, k, v = st[h]
                        s = lax.dot_general(q, k, nt, preferred_element_type=f32)
                        st[h] = (s, v)
                    h = hh - LAG2
                    if 0 <= h < H:
                        s, v = st.pop(h)
                        s = jnp.minimum(s * (scale * L2E), lim)
                        mx = jnp.max(s, axis=-1, keepdims=True)
                        e = jnp.exp2(s - mx)
                        l = jnp.sum(e, axis=-1, keepdims=True)
                        o = jnp.dot(e.astype(bf16), v, preferred_element_type=f32) * recip(l)
                        o_s[h * R:h * R + n, :] = o.astype(bf16)
                    for g in range(NG):
                        if when[g] == hh:
                            wo_group(g)

                out = jnp.concatenate([res[cc] for cc in range(CT)], axis=1)
                if mode == 'full':
                    prev_s[...] = out[0:2 * SEG]
                    newm = out[2 * SEG:]
                elif mode == 'e1':
                    prev_s[0:SEG, :] = out[0:SEG]
                    rowi = lax.broadcasted_iota(i32, (2 * M, D), 0)
                    newm = jnp.where(rowi >= M, mem0_2, out[SEG:])
                else:
                    prev_s[SEG:2 * SEG, :] = out[0:SEG]
                    newm = out[SEG:]
                if need_xn1:
                    put_lhs(0, xn1)
                if not first:
                    put_lhs(SEG, xn2)
                put_lhs(2 * SEG, newm.astype(bf16))
                if mode != 'e1':
                    @pl.when(j >= 3)
                    def _():
                        out_copy(j - 3).start()
                return c
            return step

        make_step('e1', 'all' if ALLPRE else True)(0, 0)
        make_step('e1', True)(1, 0)
        lax.fori_loop(2, NP, make_step('full', True), 0)
        for c in conv_copies(1):
            c.wait()
        x_copy[1].wait()
        lax.fori_loop(NP, NP + NU, make_step('full', False, UPS), 0)
        lax.fori_loop(NP + NU, NSEG, make_step('full'), 0)
        lax.fori_loop(NSEG, NSEG + 2, make_step('e2'), 0)
        post(NSEG + 2, do1=False)
        out_copy(NSEG - 1).start()
        pltpu.make_async_copy(out_s, out_hbm, sems.at[3, 7]).wait()

    return kernel


def build(S=2048, D=640, H=32, DH=128, M=8, SEG=32, KS=4, lags=(2, 4), flags=None, **opt):
    R = 2 * SEG + 2 * M
    CT = D // LANES
    NB = S // BLK
    HP = H // 2
    NP, EB, UPS, NU = _plan(S, D, SEG, opt)
    hbm = pl.BlockSpec(memory_space=pl.ANY)
    V = pltpu.VMEM
    scratch = [
        V((M, D), bf16), V((KS, D), bf16), V((D,), bf16), V((NFFT, BLK), bf16), V((BLK, NFFT), bf16),
        V((S, D), bf16),
        V((S, D), bf16),
        V((S, D), bf16),
        V((D, S), bf16),
        V((3 * HP, D, LANES), u32),
        V((3, H, D // 2, LANES), u32),
        V((H * DH, D), bf16),
        V((CT, S, LANES), f32),
        V((max(UPS, EB), BLK + 16, LANES), f32),
        V((CT, 8, LANES), f32),
        V((CT * NB, opt.get('xs', NFFT + 32), LANES), f32),
        V((CT * (NB + 1) + NB - 1, NFFT, LANES), f32),
        V((CT, NFFT, LANES), f32),
        V((CT, R, LANES), bf16),
        V((S + SEG, D), f32),
        V((2 * SEG, D), f32),
        V((H * R + max(UPS, EB) * NFFT, DH), bf16),
        V((S, D), bf16),
        V((CT, R, LANES), f32),
        V((CT, NP * SEG + 2 * M * opt.get('allpre', True), LANES), bf16),
        V((3, H, NP * SEG + 2 * M * opt.get('allpre', True), DH), bf16),
        pltpu.SemaphoreType.DMA((7, 16)),
    ]
    return pl.pallas_call(
        _make_kernel(S, D, H, DH, M, SEG, KS, lags, opt),
        out_shape=jax.ShapeDtypeStruct((S, D), bf16),
        in_specs=[hbm] * 13,
        out_specs=hbm,
        scratch_shapes=scratch,
        compiler_params=pltpu.CompilerParams(vmem_limit_bytes=120 * 1024 * 1024, flags=flags),
    )


def _run(A_x, A_mem0, A_Wq, A_Wk, A_Wv, A_Wo, A_seg_len, B_q, B_k, B_v, B_shift_k, B_ssm_k, B_ssm_D):
    kw = dict(gr=8,uspan=(2,35),uwd=4,fstep=2,ugap=3,alags=(0,8),eclag=(2,3),na=9)
    B, S, D = A_x.shape
    H, DH = A_Wq.shape[1:]
    M = A_mem0.shape[1]
    fwd, inv = _dft_consts()
    call = build(S, D, H, DH, M, int(A_seg_len), B_shift_k.shape[1], **kw)
    out = call(A_x.reshape(S, D), A_mem0.reshape(M, D), A_Wq, A_Wk, A_Wv, A_Wo.reshape(H * DH, D),
               B_k.reshape(S, D), B_v.reshape(S, D), B_shift_k.T, B_ssm_k, B_ssm_D,
               fwd.astype(bf16), inv.astype(bf16))
    return out.reshape(B, S, D)


@functools.partial(jax.jit, static_argnames=('A_seg_len',))
def pallas_interleave_layers__memory_aug_recurrent_mem_tr__ssm_conv_h3__prompt_kernel(
    A_x, A_mem0, A_Wq, A_Wk, A_Wv, A_Wo, A_seg_len, B_q, B_k, B_v, B_shift_k, B_ssm_k, B_ssm_D,
):
    return _run(A_x, A_mem0, A_Wq, A_Wk, A_Wv, A_Wo, A_seg_len, B_q, B_k, B_v, B_shift_k, B_ssm_k, B_ssm_D)
```

```python
import functools

import numpy as np
import jax
import jax.numpy as jnp
from jax import lax
import jax.experimental.pallas as pl
import jax.experimental.pallas.tpu as pltpu

bf16, f32, u32, i32 = jnp.bfloat16, jnp.float32, jnp.uint32, jnp.int32

LANES = 128
BLK = 128
NFFT = 2 * BLK
L2E = 1.4426950408889634
NT = (((1,), (1,)), ((), ()))

NP = 9
EB = 4
UPS = 2
GR = 8
XO, XS = 16, NFFT + 32

PIPE = {'full': (2, 4, 8), 'units': (2, 4, 4), 'pre': (3, 6, 8), 'edge': (3, 6, 12), 'first': (0, 8, 12)}
HG = 2


def _dft_consts():
    f = np.arange(BLK, dtype=np.float64)[:, None] + 0.5
    m = np.arange(BLK, dtype=np.float64)[None, :]
    ang = 2.0 * np.pi * f * m / NFFT
    fwd = np.concatenate([np.cos(ang), -np.sin(ang)], axis=0)
    inv = np.concatenate([np.cos(ang).T, -np.sin(ang).T], axis=1) * (2.0 / NFFT)
    return fwd.astype(bf16), inv.astype(bf16)


def _ln(x):
    m = jnp.mean(x, axis=-1, keepdims=True)
    c = x - m
    v = jnp.mean(c * c, axis=-1, keepdims=True)
    return c * lax.rsqrt(v + 1e-5)


def _as16(words):
    return pltpu.bitcast(words, bf16)


def _ds(start, size, align):
    if isinstance(start, int):
        return pl.ds(start, size)
    return pl.ds(pl.multiple_of(start, align), size)


def _clip(j, lo, hi):
    return min(max(j, lo), hi) if isinstance(j, int) else jnp.clip(j, lo, hi)


def _make_kernel(S, D, H, DH, M, SEG, KS):
    NSEG = S // SEG
    R = 2 * SEG + 2 * M
    RE = SEG + 2 * M
    CT = D // LANES
    NB = S // BLK
    HP = H // 2
    NU = (NB - EB) * CT // UPS
    GP = NB - 1
    PR = NP * SEG
    XHEAD = (NP + 2) * SEG
    ZB = H * R
    scale = DH ** -0.5

    def kernel(x_hbm, mem0_hbm, wq_hbm, wk_hbm, wv_hbm, wo_hbm, k_hbm, v_hbm, shift_hbm, ssm_hbm, ssmd_hbm,
               fwd_hbm, inv_hbm, out_hbm,
               mem0_s, shift_s, ssmd_s, fwd_s, inv_s,
               x_s, k_s, v_s, ssm_s, stage_s, w_s, wo_s, y_s, kq_s, par_s, xg_s, gg_s, kr_s,
               lhs_s, x2_s, prev_s, o_s, out_s, acc_s, xn_s, pre_s, sems):
        w32 = [r.bitcast(u32) for r in (wq_hbm, wk_hbm, wv_hbm)]
        small = [pltpu.make_async_copy(a, b, sems.at[3, 8 + i]) for i, (a, b) in enumerate(
            [(shift_hbm, shift_s), (ssmd_hbm, ssmd_s), (fwd_hbm, fwd_s), (inv_hbm, inv_s), (mem0_hbm, mem0_s)])]
        x_copy = [pltpu.make_async_copy(x_hbm.at[a:b], x_s.at[a:b], sems.at[3, i])
                  for i, (a, b) in enumerate([(0, XHEAD), (XHEAD, S)])]
        wo_copy = pltpu.make_async_copy(wo_hbm, wo_s, sems.at[3, 2])

        def conv_copies(part):
            sl = slice(0, EB * BLK) if part == 0 else slice(EB * BLK, S)
            return (pltpu.make_async_copy(k_hbm.at[sl], k_s.at[sl], sems.at[0, part]),
                    pltpu.make_async_copy(v_hbm.at[sl], v_s.at[sl], sems.at[1, part]),
                    pltpu.make_async_copy(ssm_hbm.at[:, sl], ssm_s.at[:, sl], sems.at[2, part]))

        for c in small:
            c.start()
        x_copy[0].start()
        for i in range(HP):
            for m in range(3):
                pltpu.make_async_copy(w32[m].at[:, i, :], stage_s.at[m * HP + i], sems.at[4 + m, i]).start()
        for c in conv_copies(0):
            c.start()
        wo_copy.start()
        for c in conv_copies(1):
            c.start()
        x_copy[1].start()

        xn32, lhs32, o32 = xn_s.bitcast(u32), lhs_s.bitcast(u32), o_s.bitcast(u32)

        for c in small:
            c.wait()
        x_copy[0].wait()
        for r0 in range(0, PR, SEG):
            xn = _ln(x_s[r0:r0 + SEG, :].astype(f32)).astype(bf16)
            for cc in range(CT):
                xn_s[cc, r0:r0 + SEG, :] = xn[:, cc * LANES:(cc + 1) * LANES]
        mem0 = mem0_s[...]
        mem0_2 = jnp.concatenate([mem0, mem0], axis=0)
        for cc in range(CT):
            xn_s[cc, PR:PR + 2 * M, :] = mem0_2[:, cc * LANES:(cc + 1) * LANES]

        def head_pair(i, carry):
            lo_mask = jnp.full((64, LANES), 0xFFFF, u32)
            for m in range(3):
                pltpu.make_async_copy(stage_s.at[m * HP + i], stage_s.at[m * HP + i], sems.at[4 + m, i]).wait()
            for m in range(3):
                for c0 in range(0, D // 2, 64):
                    ev = stage_s[m * HP + i, pl.ds(2 * c0, 64, stride=2), :]
                    od = stage_s[m * HP + i, pl.ds(2 * c0 + 1, 64, stride=2), :]
                    w_s[m, 2 * i, pl.ds(c0, 64), :] = (ev & lo_mask) | (od << 16)
                    w_s[m, 2 * i + 1, pl.ds(c0, 64), :] = (ev >> 16) | (od & ~lo_mask)
            lhs = jnp.concatenate([_as16(xn32[cc]) for cc in range(CT)], axis=1)
            for m in range(3):
                for hh in range(2):
                    r = jnp.dot(lhs, _as16(w_s[m, 2 * i + hh]), preferred_element_type=f32)
                    pre_s[m, 2 * i + hh] = r.astype(bf16)
            return carry

        lax.fori_loop(0, HP, head_pair, 0)

        shift_t = shift_s[...].astype(f32)
        for ct in range(CT):
            cs = slice(ct * LANES, (ct + 1) * LANES)
            par_s[ct, 0:KS, :] = shift_t[:, cs]
            par_s[ct, KS:KS + 1, :] = ssmd_s[cs].astype(f32).reshape(1, LANES)

        def conv_front(a, ct, slot, kprev=None, keep=True):
            fwd = fwd_s[...]
            cs = _ds(ct * LANES, LANES, LANES)
            r = _ds(a * BLK, BLK, BLK)
            first = isinstance(a, int) and a == 0
            if first:
                kq_s[slot, 0:16, :] = jnp.zeros((16, LANES), f32)
                kq_s[slot, 16:, :] = k_s[r, cs].astype(f32)
            else:
                kq_s[slot] = k_s[_ds(a * BLK - 16, BLK + 16, 16), cs].astype(f32)
            acc = None
            for t in range(KS):
                term = kq_s[slot, 16 - t:16 - t + BLK, :] * par_s[ct, t:t + 1, :]
                acc = term if acc is None else acc + term
            kv = (acc * v_s[r, cs].astype(f32)).astype(bf16)
            y_s[ct, r, :] = kv.astype(f32) * par_s[ct, KS:KS + 1, :]
            xg_s[ct * NB + a, XO:XO + NFFT, :] = jnp.dot(fwd, kv, preferred_element_type=f32)
            kf = lax.dot_general(fwd, ssm_s[cs, r], NT, preferred_element_type=f32)
            g = GP + ct * (NB + 1) + a
            if first:
                gg_s[g] = kf
            else:
                rows = lax.broadcasted_iota(i32, (BLK, LANES), 0)
                sgn = jnp.where((rows & 1) == 0, 1.0, -1.0).astype(f32)
                if kprev is None:
                    pr, pi = kr_s[ct, 0:BLK, :], kr_s[ct, BLK:NFFT, :]
                else:
                    pr, pi = kprev[0:BLK], kprev[BLK:NFFT]
                gg_s[g, 0:BLK, :] = kf[0:BLK] - sgn * pi
                gg_s[g, BLK:NFFT, :] = kf[BLK:NFFT] + sgn * pr
            if keep:
                kr_s[ct] = kf
            return kf

        def conv_mac(a, ct, nout, zero, slot, gr):
            static = isinstance(a, int)
            g0 = GP + ct * (NB + 1) + a
            for g in range(BLK // gr):
                re = slice(g * gr, (g + 1) * gr)
                im = slice(BLK + g * gr, BLK + (g + 1) * gr)
                z = [None] * nout
                win = {}
                for b in range(a + nout if static else NB):
                    xr = xg_s[ct * NB + b, XO + re.start:XO + re.stop, :]
                    xi = xg_s[ct * NB + b, XO + im.start:XO + im.stop, :]
                    for o in range(nout):
                        c = o - b
                        if static and a + c < 0:
                            continue
                        if c not in win:
                            win[c] = (gg_s[g0 + c, re, :], gg_s[g0 + c, im, :])
                        gre, gim = win[c]
                        if z[o] is None:
                            z[o] = (gre * xr - gim * xi, gre * xi + gim * xr)
                        else:
                            z[o] = (z[o][0] + gre * xr - gim * xi, z[o][1] + gre * xi + gim * xr)
                    win.pop(nout - 1 - b, None)
                for o in range(nout):
                    zb = ZB + (slot + o) * NFFT + zero
                    o_s[_ds(zb + re.start, gr, gr), :] = z[o][0].astype(bf16)
                    o_s[_ds(zb + im.start, gr, gr), :] = z[o][1].astype(bf16)
                yield

        def conv_back(a, ct, slot):
            r = _ds(a * BLK, BLK, BLK)
            z = _as16(o32[(ZB + slot * NFFT) // 2:(ZB + (slot + 1) * NFFT) // 2, :])
            y_s[ct, r, :] = y_s[ct, r, :] + jnp.dot(inv_s[...], z, preferred_element_type=f32)

        def conv_unit(a, ct, zero):
            for o in range(UPS):
                conv_front(a + o, ct, o)
                yield
            yield from conv_mac(a, ct, UPS, zero, 0, GR)
            for o in range(UPS):
                conv_back(a + o, ct, o)
            yield

        for c in conv_copies(0):
            c.wait()
        for ct in range(CT):
            kprev = None
            for t in range(EB + 3):
                if t < EB:
                    kprev = conv_front(t, ct, t % UPS, kprev, keep=(t == EB - 1))
                if 0 <= t - 2 < EB:
                    for _ in conv_mac(t - 2, ct, 1, 0, (t - 2) % UPS, 16):
                        pass
                if 0 <= t - 3 < EB:
                    conv_back(t - 3, ct, (t - 3) % UPS)

        def rows(seg):
            return _ds(seg * SEG, SEG, SEG)

        def load_y(seg):
            return jnp.concatenate([y_s[ct, rows(seg), :] for ct in range(CT)], axis=1)

        def put_lhs(r0, val):
            for cc in range(CT):
                lhs_s[cc, r0:r0 + val.shape[0], :] = val[:, cc * LANES:(cc + 1) * LANES]

        def out_copy(seg):
            return pltpu.make_async_copy(out_s.at[rows(seg)], out_hbm.at[rows(seg)], sems.at[3, 7])

        put_lhs(0, jnp.zeros((2 * SEG, D), bf16))
        put_lhs(2 * SEG, mem0_2)
        x2_s[0:SEG, :] = jnp.zeros((SEG, D), f32)
        prev_s[...] = jnp.zeros((2 * SEG, D), f32)

        def post(j, do1=True, do2=True):
            xn2 = None
            if do2:
                sb = _clip(j - 3, 0, NSEG - 1)
                x3 = x2_s[rows(sb), :] + prev_s[SEG:2 * SEG, :]
                out_s[rows(sb), :] = (x3 + _ln(x3) * load_y(sb)).astype(bf16)
            if do1:
                sa = _clip(j - 1, 0, NSEG - 1)
                x1 = x_s[rows(sa), :].astype(f32) + prev_s[0:SEG, :]
                x2 = x1 + _ln(x1) * load_y(sa)
                x2_s[rows(_clip(j - 1, 0, NSEG)), :] = x2
                xn2 = _ln(x2).astype(bf16)
            return xn2

        def limits(n, live):
            ri = lax.broadcasted_iota(i32, (n, n), 0)
            ci = lax.broadcasted_iota(i32, (n, n), 1)
            ntok = n - 2 * M

            def layer(i):
                if live is None:
                    return jnp.where(i < ntok, i // SEG, (i - ntok) // M)
                return jnp.where(i < ntok, 0, jnp.where((i - ntok) // M == live, 0, 1))
            ok = (layer(ri) == layer(ci)) & ((ri >= ntok) | (ci >= ntok) | (ri >= ci))
            return jnp.where(ok, 3.0e38, -1e9 * L2E).astype(f32)

        def make_step(kind):
            both = kind in ('pre', 'units', 'full')
            n = R if both else RE
            lag1, lag2, wdel = PIPE[{'edge1': 'edge', 'edge2': 'edge'}.get(kind, kind)]
            ngroups = H // HG
            if kind in ('units', 'full'):
                spans = [(0, R)]
            elif kind == 'pre':
                spans = [(SEG, R)]
            elif kind == 'edge2':
                spans = [(SEG, 2 * SEG), (2 * SEG, R)]
            else:
                spans = [(2 * SEG, R)]

            def step(j, carry):
                lim = limits(n, None if both else int(kind == 'edge2'))
                lhs = None
                if kind != 'first':
                    lhs = jnp.concatenate(
                        [_as16(jnp.concatenate([lhs32[cc, a // 2:b // 2, :] for a, b in spans], axis=0))
                         for cc in range(CT)], axis=1)

                def proj(m, h):
                    if kind == 'first':
                        return jnp.concatenate([pre_s[m, h, rows(j), :], pre_s[m, h, PR:PR + 2 * M, :]], axis=0)
                    r = jnp.dot(lhs, _as16(w_s[m, h]), preferred_element_type=f32).astype(bf16)
                    if kind in ('pre', 'edge1'):
                        r = jnp.concatenate([pre_s[m, h, rows(j), :], r], axis=0)
                    return r

                side = {}
                if kind == 'units':
                    u = j - NP
                    gen = conv_unit(EB + (u // CT) * UPS, u % CT, jnp.minimum(j, 0))
                    nmac = BLK // GR
                    m0 = 2 + 2 * UPS + 3
                    at = [2 + 2 * o for o in range(UPS)]
                    at += [int(round(m0 + p * (H + lag2 - 2 - m0) / (nmac - 1))) for p in range(nmac)]
                    at.append(at[-1] + 1)
                    for hh in at:
                        side.setdefault(hh, []).append(gen.__next__)
                if kind == 'pre':
                    nz = NB - EB
                    nx, ng = CT * nz, GP + CT * (nz + 1)
                    px, pg = -(-nx // (NP - 2)), -(-ng // (NP - 2))
                    zblk = jnp.zeros((NFFT, LANES), f32)

                    def zero_x(q):
                        kx = jnp.minimum((j - 2) * px + q, nx - 1)
                        xg_s[(kx // nz) * NB + EB + kx % nz, XO:XO + NFFT, :] = zblk

                    def zero_g(q):
                        kg = jnp.minimum((j - 2) * pg + q, ng - 1)
                        kk = jnp.maximum(kg - GP, 0)
                        gg_s[jnp.where(kg < GP, kg, GP + (kk // (nz + 1)) * (NB + 1) + EB + kk % (nz + 1))] = zblk
                    jobs = [functools.partial(zero_x, q) for q in range(px)]
                    jobs += [functools.partial(zero_g, q) for q in range(pg)]
                    for q, job in enumerate(jobs):
                        side.setdefault(q * H // len(jobs), []).append(job)

                xn2 = None if kind == 'first' else post(j, do2=(kind != 'edge1'))
                if both:
                    xn1 = _ln(x_s[rows(_clip(j + 1, 0, NSEG - 1)), :].astype(f32)).astype(bf16)

                live, res = {}, {}

                def out_proj(g):
                    ob = jnp.concatenate([_as16(o32[h * R // 2:(h * R + n) // 2, :])
                                          for h in range(g * HG, (g + 1) * HG)], axis=1)
                    for cc in range(CT):
                        t = jnp.dot(ob, wo_s[g * HG * DH:(g + 1) * HG * DH, cc * LANES:(cc + 1) * LANES],
                                    preferred_element_type=f32)
                        if g > 0:
                            t = t + acc_s[cc, 0:n, :]
                        if g < ngroups - 1:
                            acc_s[cc, 0:n, :] = t
                        else:
                            res[cc] = t

                for hh in range(H + lag2):
                    for job in side.get(hh, []):
                        job()
                    if hh < H:
                        live[hh] = (proj(0, hh), proj(1, hh), proj(2, hh))
                    h = hh - lag1
                    if 0 <= h < H:
                        q, k, v = live[h]
                        live[h] = (lax.dot_general(q, k, NT, preferred_element_type=f32), v)
                    h = hh - lag2
                    if 0 <= h < H:
                        s, v = live.pop(h)
                        s = jnp.minimum(s * (scale * L2E), lim)
                        e = jnp.exp2(s - jnp.max(s, axis=-1, keepdims=True))
                        l = jnp.sum(e, axis=-1, keepdims=True)
                        rl = pl.reciprocal(l, approx=True)
                        rl = rl * (2.0 - l * rl)
                        o = jnp.dot(e.astype(bf16), v, preferred_element_type=f32) * rl
                        o_s[h * R:h * R + n, :] = o.astype(bf16)
                    for g in range(ngroups):
                        if min((g + 1) * HG - 1 + lag2 + wdel, H + lag2 - 1) == hh:
                            out_proj(g)

                out = jnp.concatenate([res[cc] for cc in range(CT)], axis=1)
                if both:
                    prev_s[...] = out[0:2 * SEG]
                    put_lhs(0, xn1)
                elif kind == 'edge2':
                    prev_s[SEG:2 * SEG, :] = out[0:SEG]
                else:
                    prev_s[0:SEG, :] = out[0:SEG]
                newm = out[n - 2 * M:]
                if kind in ('first', 'edge1'):
                    mrow = lax.broadcasted_iota(i32, (2 * M, D), 0)
                    newm = jnp.where(mrow >= M, mem0_2.astype(f32), newm)
                if xn2 is not None:
                    put_lhs(SEG, xn2)
                put_lhs(2 * SEG, newm.astype(bf16))
                if kind == 'pre':
                    @pl.when(j >= 3)
                    def _():
                        out_copy(j - 3).start()
                elif kind not in ('first', 'edge1'):
                    out_copy(j - 3).start()
                return carry
            return step

        wo_copy.wait()
        make_step('first')(0, 0)
        make_step('edge1')(1, 0)
        lax.fori_loop(2, NP, make_step('pre'), 0)
        for c in conv_copies(1):
            c.wait()
        x_copy[1].wait()
        units_step = make_step('units')
        lax.fori_loop(0, NU, lambda i, c: units_step(i + NP, c), 0)
        lax.fori_loop(NP + NU, NSEG, make_step('full'), 0)
        lax.fori_loop(NSEG, NSEG + 2, make_step('edge2'), 0)
        post(NSEG + 2, do1=False)
        out_copy(NSEG - 1).start()
        pltpu.make_async_copy(out_s, out_hbm, sems.at[3, 7]).wait()

    return kernel


def _build(S, D, H, DH, M, SEG, KS):
    NSEG, CT, NB, HP = S // SEG, D // LANES, S // BLK, H // 2
    R = 2 * SEG + 2 * M
    NU = (NB - EB) * CT // UPS
    assert DH == LANES and D % LANES == 0 and S % BLK == 0 and SEG % 16 == 0 and M % 8 == 0
    assert H % 2 == 0 and R <= LANES and KS < 8 and BLK % SEG == 0
    assert (NB - EB) * CT % UPS == 0 and EB % UPS == 0 and 2 < NP and NP + NU <= NSEG
    assert NP + CT <= EB * (BLK // SEG)
    hbm = pl.BlockSpec(memory_space=pl.ANY)
    V = pltpu.VMEM
    scratch = [
        V((M, D), bf16), V((KS, D), bf16), V((D,), bf16), V((NFFT, BLK), bf16), V((BLK, NFFT), bf16),
        V((S, D), bf16),
        V((S, D), bf16),
        V((S, D), bf16),
        V((D, S), bf16),
        V((3 * HP, D, LANES), u32),
        V((3, H, D // 2, LANES), u32),
        V((H * DH, D), bf16),
        V((CT, S, LANES), f32),
        V((UPS, BLK + 16, LANES), f32),
        V((CT, 8, LANES), f32),
        V((CT * NB, XS, LANES), f32),
        V((CT * (NB + 1) + NB - 1, NFFT, LANES), f32),
        V((CT, NFFT, LANES), f32),
        V((CT, R, LANES), bf16),
        V((S + SEG, D), f32),
        V((2 * SEG, D), f32),
        V((H * R + UPS * NFFT, DH), bf16),
        V((S, D), bf16),
        V((CT, R, LANES), f32),
        V((CT, NP * SEG + 2 * M, LANES), bf16),
        V((3, H, NP * SEG + 2 * M, DH), bf16),
        pltpu.SemaphoreType.DMA((7, 16)),
    ]
    return pl.pallas_call(
        _make_kernel(S, D, H, DH, M, SEG, KS),
        out_shape=jax.ShapeDtypeStruct((S, D), bf16),
        in_specs=[hbm] * 13,
        out_specs=hbm,
        scratch_shapes=scratch,
        compiler_params=pltpu.CompilerParams(vmem_limit_bytes=120 * 1024 * 1024),
    )


@functools.partial(jax.jit, static_argnames=('A_seg_len',))
def pallas_interleave_layers__memory_aug_recurrent_mem_tr__ssm_conv_h3__prompt_kernel(
    A_x: jax.Array,
    A_mem0: jax.Array,
    A_Wq: jax.Array,
    A_Wk: jax.Array,
    A_Wv: jax.Array,
    A_Wo: jax.Array,
    A_seg_len: int,
    B_q: jax.Array,
    B_k: jax.Array,
    B_v: jax.Array,
    B_shift_k: jax.Array,
    B_ssm_k: jax.Array,
    B_ssm_D: jax.Array,
):
    del B_q
    B, S, D = A_x.shape
    H, DH = A_Wq.shape[1:]
    M = A_mem0.shape[1]
    assert B == 1
    fwd, inv = _dft_consts()
    call = _build(S, D, H, DH, M, int(A_seg_len), B_shift_k.shape[1])
    out = call(A_x.reshape(S, D), A_mem0.reshape(M, D), A_Wq, A_Wk, A_Wv, A_Wo.reshape(H * DH, D),
               B_k.reshape(S, D), B_v.reshape(S, D), B_shift_k.T, B_ssm_k, B_ssm_D, fwd, inv)
    return out.reshape(B, S, D)
```

```python
import functools

import numpy as np
import jax
import jax.numpy as jnp
from jax import lax
import jax.experimental.pallas as pl
import jax.experimental.pallas.tpu as pltpu

bf16, f32, u32, i32 = jnp.bfloat16, jnp.float32, jnp.uint32, jnp.int32

LANES = 128
BLK = 128
NFFT = 2 * BLK
L2E = 1.4426950408889634
NT = (((1,), (1,)), ((), ()))

NP = 10
EB = 4
UPS = 2
GR = 8
XO, XS = 16, NFFT + 32

PIPE = {'full': (2, 4, 8), 'units': (2, 4, 4), 'pre': (3, 6, 8), 'edge': (3, 6, 12), 'first': (0, 8, 12)}
HG = 2


def _dft_consts():
    f = np.arange(BLK, dtype=np.float64)[:, None] + 0.5
    m = np.arange(BLK, dtype=np.float64)[None, :]
    ang = 2.0 * np.pi * f * m / NFFT
    fwd = np.concatenate([np.cos(ang), -np.sin(ang)], axis=0)
    inv = np.concatenate([np.cos(ang).T, -np.sin(ang).T], axis=1) * (2.0 / NFFT)
    return fwd.astype(bf16), inv.astype(bf16)


def _ln(x):
    m = jnp.mean(x, axis=-1, keepdims=True)
    c = x - m
    v = jnp.mean(c * c, axis=-1, keepdims=True)
    return c * lax.rsqrt(v + 1e-5)


def _as16(words):
    return pltpu.bitcast(words, bf16)


def _ds(start, size, align):
    if isinstance(start, int):
        return pl.ds(start, size)
    return pl.ds(pl.multiple_of(start, align), size)


def _clip(j, lo, hi):
    return min(max(j, lo), hi) if isinstance(j, int) else jnp.clip(j, lo, hi)


def _make_kernel(S, D, H, DH, M, SEG, KS):
    NSEG = S // SEG
    R = 2 * SEG + 2 * M
    RE = SEG + 2 * M
    CT = D // LANES
    NB = S // BLK
    HP = H // 2
    NU = (NB - EB) * CT // UPS
    GP = NB - 1
    PR = NP * SEG
    XHEAD = (NP + 2) * SEG
    ZB = H * R
    scale = DH ** -0.5

    def kernel(x_hbm, mem0_hbm, wq_hbm, wk_hbm, wv_hbm, wo_hbm, k_hbm, v_hbm, shift_hbm, ssm_hbm, ssmd_hbm,
               fwd_hbm, inv_hbm, out_hbm,
               mem0_s, shift_s, ssmd_s, fwd_s, inv_s,
               x_s, k_s, v_s, ssm_s, stage_s, w_s, wo_s, y_s, kq_s, par_s, xg_s, gg_s, kr_s,
               lhs_s, x2_s, prev_s, o_s, out_s, acc_s, xn_s, pre_s, sems):
        w32 = [r.bitcast(u32) for r in (wq_hbm, wk_hbm, wv_hbm)]
        small = [pltpu.make_async_copy(a, b, sems.at[3, 8 + i]) for i, (a, b) in enumerate(
            [(shift_hbm, shift_s), (ssmd_hbm, ssmd_s), (fwd_hbm, fwd_s), (inv_hbm, inv_s), (mem0_hbm, mem0_s)])]
        x_copy = [pltpu.make_async_copy(x_hbm.at[a:b], x_s.at[a:b], sems.at[3, i])
                  for i, (a, b) in enumerate([(0, XHEAD), (XHEAD, S)])]
        wo_copy = pltpu.make_async_copy(wo_hbm, wo_s, sems.at[3, 2])

        def conv_copies(part):
            sl = slice(0, EB * BLK) if part == 0 else slice(EB * BLK, S)
            return (pltpu.make_async_copy(k_hbm.at[sl], k_s.at[sl], sems.at[0, part]),
                    pltpu.make_async_copy(v_hbm.at[sl], v_s.at[sl], sems.at[1, part]),
                    pltpu.make_async_copy(ssm_hbm.at[:, sl], ssm_s.at[:, sl], sems.at[2, part]))

        for c in small:
            c.start()
        x_copy[0].start()
        for i in range(HP):
            for m in range(3):
                pltpu.make_async_copy(w32[m].at[:, i, :], stage_s.at[m * HP + i], sems.at[4 + m, i]).start()
        for c in conv_copies(0):
            c.start()
        wo_copy.start()
        for c in conv_copies(1):
            c.start()
        x_copy[1].start()

        xn32, lhs32, o32 = xn_s.bitcast(u32), lhs_s.bitcast(u32), o_s.bitcast(u32)

        for c in small:
            c.wait()
        x_copy[0].wait()
        for r0 in range(0, PR, SEG):
            xn = _ln(x_s[r0:r0 + SEG, :].astype(f32)).astype(bf16)
            for cc in range(CT):
                xn_s[cc, r0:r0 + SEG, :] = xn[:, cc * LANES:(cc + 1) * LANES]
        mem0 = mem0_s[...]
        mem0_2 = jnp.concatenate([mem0, mem0], axis=0)
        for cc in range(CT):
            xn_s[cc, PR:PR + 2 * M, :] = mem0_2[:, cc * LANES:(cc + 1) * LANES]

        def head_pair(i, carry):
            lo_mask = jnp.full((64, LANES), 0xFFFF, u32)
            for m in range(3):
                pltpu.make_async_copy(stage_s.at[m * HP + i], stage_s.at[m * HP + i], sems.at[4 + m, i]).wait()
            for m in range(3):
                for c0 in range(0, D // 2, 64):
                    ev = stage_s[m * HP + i, pl.ds(2 * c0, 64, stride=2), :]
                    od = stage_s[m * HP + i, pl.ds(2 * c0 + 1, 64, stride=2), :]
                    w_s[m, 2 * i, pl.ds(c0, 64), :] = (ev & lo_mask) | (od << 16)
                    w_s[m, 2 * i + 1, pl.ds(c0, 64), :] = (ev >> 16) | (od & ~lo_mask)
            lhs = jnp.concatenate([_as16(xn32[cc]) for cc in range(CT)], axis=1)
            for m in range(3):
                for hh in range(2):
                    r = jnp.dot(lhs, _as16(w_s[m, 2 * i + hh]), preferred_element_type=f32)
                    pre_s[m, 2 * i + hh] = r.astype(bf16)
            return carry

        lax.fori_loop(0, HP, head_pair, 0)

        shift_t = shift_s[...].astype(f32)
        for ct in range(CT):
            cs = slice(ct * LANES, (ct + 1) * LANES)
            par_s[ct, 0:KS, :] = shift_t[:, cs]
            par_s[ct, KS:KS + 1, :] = ssmd_s[cs].astype(f32).reshape(1, LANES)

        def conv_front(a, ct, slot):
            fwd = fwd_s[...]
            cs = _ds(ct * LANES, LANES, LANES)
            r = _ds(a * BLK, BLK, BLK)
            first = isinstance(a, int) and a == 0
            if first:
                kq_s[slot, 0:16, :] = jnp.zeros((16, LANES), f32)
                kq_s[slot, 16:, :] = k_s[r, cs].astype(f32)
            else:
                kq_s[slot] = k_s[_ds(a * BLK - 16, BLK + 16, 16), cs].astype(f32)
            acc = None
            for t in range(KS):
                term = kq_s[slot, 16 - t:16 - t + BLK, :] * par_s[ct, t:t + 1, :]
                acc = term if acc is None else acc + term
            kv = (acc * v_s[r, cs].astype(f32)).astype(bf16)
            y_s[ct, r, :] = kv.astype(f32) * par_s[ct, KS:KS + 1, :]
            xg_s[ct * NB + a, XO:XO + NFFT, :] = jnp.dot(fwd, kv, preferred_element_type=f32)
            kf = lax.dot_general(fwd, ssm_s[cs, r], NT, preferred_element_type=f32)
            g = GP + ct * (NB + 1) + a
            if first:
                gg_s[g] = kf
            else:
                rows = lax.broadcasted_iota(i32, (BLK, LANES), 0)
                sgn = jnp.where((rows & 1) == 0, 1.0, -1.0).astype(f32)
                gg_s[g, 0:BLK, :] = kf[0:BLK] - sgn * kr_s[ct, BLK:NFFT, :]
                gg_s[g, BLK:NFFT, :] = kf[BLK:NFFT] + sgn * kr_s[ct, 0:BLK, :]
            kr_s[ct] = kf

        def conv_mac(a, ct, nout, zero, slot, gr):
            static = isinstance(a, int)
            g0 = GP + ct * (NB + 1) + a
            for g in range(BLK // gr):
                re = slice(g * gr, (g + 1) * gr)
                im = slice(BLK + g * gr, BLK + (g + 1) * gr)
                z = [None] * nout
                win = {}
                for b in range(a + nout if static else NB):
                    xr = xg_s[ct * NB + b, XO + re.start:XO + re.stop, :]
                    xi = xg_s[ct * NB + b, XO + im.start:XO + im.stop, :]
                    for o in range(nout):
                        c = o - b
                        if static and a + c < 0:
                            continue
                        if c not in win:
                            win[c] = (gg_s[g0 + c, re, :], gg_s[g0 + c, im, :])
                        gre, gim = win[c]
                        if z[o] is None:
                            z[o] = (gre * xr - gim * xi, gre * xi + gim * xr)
                        else:
                            z[o] = (z[o][0] + gre * xr - gim * xi, z[o][1] + gre * xi + gim * xr)
                    win.pop(nout - 1 - b, None)
                for o in range(nout):
                    zb = ZB + (slot + o) * NFFT + zero
                    o_s[_ds(zb + re.start, gr, gr), :] = z[o][0].astype(bf16)
                    o_s[_ds(zb + im.start, gr, gr), :] = z[o][1].astype(bf16)
                yield

        def conv_back(a, ct, slot):
            r = _ds(a * BLK, BLK, BLK)
            z = _as16(o32[(ZB + slot * NFFT) // 2:(ZB + (slot + 1) * NFFT) // 2, :])
            y_s[ct, r, :] = y_s[ct, r, :] + jnp.dot(inv_s[...], z, preferred_element_type=f32)

        def conv_unit(a, ct, zero):
            for o in range(UPS):
                conv_front(a + o, ct, o)
                yield
            yield from conv_mac(a, ct, UPS, zero, 0, GR)
            for o in range(UPS):
                conv_back(a + o, ct, o)
            yield

        def conv_early(blocks):
            def front(a, ct, slot):
                conv_front(a, ct, slot)

            def mac(a, ct, slot):
                for _ in conv_mac(a, ct, 1, 0, slot, 16):
                    pass
            units = [(a, ct, i % UPS) for i, (a, ct) in enumerate((a, ct) for a in blocks for ct in range(CT))]
            return [functools.partial(fn, *units[t - lag])
                    for t in range(len(units) + 2) for lag, fn in enumerate((front, mac, conv_back))
                    if 0 <= t - lag < len(units)]

        def rows(seg):
            return _ds(seg * SEG, SEG, SEG)

        def load_y(seg):
            return jnp.concatenate([y_s[ct, rows(seg), :] for ct in range(CT)], axis=1)

        def put_lhs(r0, val):
            for cc in range(CT):
                lhs_s[cc, r0:r0 + val.shape[0], :] = val[:, cc * LANES:(cc + 1) * LANES]

        def out_copy(seg):
            return pltpu.make_async_copy(out_s.at[rows(seg)], out_hbm.at[rows(seg)], sems.at[3, 7])

        put_lhs(0, jnp.zeros((2 * SEG, D), bf16))
        put_lhs(2 * SEG, mem0_2)
        x2_s[0:SEG, :] = jnp.zeros((SEG, D), f32)
        prev_s[...] = jnp.zeros((2 * SEG, D), f32)

        def post(j, do1=True, do2=True):
            xn2 = None
            if do2:
                sb = _clip(j - 3, 0, NSEG - 1)
                x3 = x2_s[rows(sb), :] + prev_s[SEG:2 * SEG, :]
                out_s[rows(sb), :] = (x3 + _ln(x3) * load_y(sb)).astype(bf16)
            if do1:
                sa = _clip(j - 1, 0, NSEG - 1)
                x1 = x_s[rows(sa), :].astype(f32) + prev_s[0:SEG, :]
                x2 = x1 + _ln(x1) * load_y(sa)
                x2_s[rows(_clip(j - 1, 0, NSEG)), :] = x2
                xn2 = _ln(x2).astype(bf16)
            return xn2

        def limits(n, live):
            ri = lax.broadcasted_iota(i32, (n, n), 0)
            ci = lax.broadcasted_iota(i32, (n, n), 1)
            ntok = n - 2 * M

            def layer(i):
                if live is None:
                    return jnp.where(i < ntok, i // SEG, (i - ntok) // M)
                return jnp.where(i < ntok, 0, jnp.where((i - ntok) // M == live, 0, 1))
            ok = (layer(ri) == layer(ci)) & ((ri >= ntok) | (ci >= ntok) | (ri >= ci))
            return jnp.where(ok, 3.0e38, -1e9 * L2E).astype(f32)

        def make_step(kind):
            both = kind in ('pre', 'units', 'full')
            n = R if both else RE
            lag1, lag2, wdel = PIPE[{'edge1': 'edge', 'edge2': 'edge'}.get(kind, kind)]
            ngroups = H // HG
            if kind in ('units', 'full'):
                spans = [(0, R)]
            elif kind == 'pre':
                spans = [(SEG, R)]
            elif kind == 'edge2':
                spans = [(SEG, 2 * SEG), (2 * SEG, R)]
            else:
                spans = [(2 * SEG, R)]

            def step(j, carry):
                lim = limits(n, None if both else int(kind == 'edge2'))
                lhs = None
                if kind != 'first':
                    lhs = jnp.concatenate(
                        [_as16(jnp.concatenate([lhs32[cc, a // 2:b // 2, :] for a, b in spans], axis=0))
                         for cc in range(CT)], axis=1)

                def proj(m, h):
                    if kind == 'first':
                        return jnp.concatenate([pre_s[m, h, rows(j), :], pre_s[m, h, PR:PR + 2 * M, :]], axis=0)
                    r = jnp.dot(lhs, _as16(w_s[m, h]), preferred_element_type=f32).astype(bf16)
                    if kind in ('pre', 'edge1'):
                        r = jnp.concatenate([pre_s[m, h, rows(j), :], r], axis=0)
                    return r

                side = {}
                if kind == 'units':
                    u = j - NP
                    gen = conv_unit(EB + (u // CT) * UPS, u % CT, jnp.minimum(j, 0))
                    nmac = BLK // GR
                    m0 = 2 + 2 * UPS + 3
                    at = [2 + 2 * o for o in range(UPS)]
                    at += [int(round(m0 + p * (H + lag2 - 2 - m0) / (nmac - 1))) for p in range(nmac)]
                    at.append(at[-1] + 1)
                    for hh in at:
                        side.setdefault(hh, []).append(gen.__next__)
                if kind in ('first', 'edge1'):
                    jobs = conv_early(range(0, 1) if kind == 'first' else range(1, EB))
                    for q, job in enumerate(jobs):
                        side.setdefault(q * (H + lag2) // len(jobs), []).append(job)
                if kind == 'pre':
                    nz = NB - EB
                    nx, ng = CT * nz, GP + CT * (nz + 1)
                    px, pg = -(-nx // (NP - 2)), -(-ng // (NP - 2))
                    zblk = jnp.zeros((NFFT, LANES), f32)

                    def zero_x(q):
                        kx = jnp.minimum((j - 2) * px + q, nx - 1)
                        xg_s[(kx // nz) * NB + EB + kx % nz, XO:XO + NFFT, :] = zblk

                    def zero_g(q):
                        kg = jnp.minimum((j - 2) * pg + q, ng - 1)
                        kk = jnp.maximum(kg - GP, 0)
                        gg_s[jnp.where(kg < GP, kg, GP + (kk // (nz + 1)) * (NB + 1) + EB + kk % (nz + 1))] = zblk
                    jobs = [functools.partial(zero_x, q) for q in range(px)]
                    jobs += [functools.partial(zero_g, q) for q in range(pg)]
                    for q, job in enumerate(jobs):
                        side.setdefault(q * H // len(jobs), []).append(job)

                xn2 = None if kind == 'first' else post(j, do2=(kind != 'edge1'))
                if both:
                    xn1 = _ln(x_s[rows(_clip(j + 1, 0, NSEG - 1)), :].astype(f32)).astype(bf16)

                live, res = {}, {}

                def out_proj(g):
                    ob = jnp.concatenate([_as16(o32[h * R // 2:(h * R + n) // 2, :])
                                          for h in range(g * HG, (g + 1) * HG)], axis=1)
                    for cc in range(CT):
                        t = jnp.dot(ob, wo_s[g * HG * DH:(g + 1) * HG * DH, cc * LANES:(cc + 1) * LANES],
                                    preferred_element_type=f32)
                        if g > 0:
                            t = t + acc_s[cc, 0:n, :]
                        if g < ngroups - 1:
                            acc_s[cc, 0:n, :] = t
                        else:
                            res[cc] = t

                for hh in range(H + lag2):
                    for job in side.get(hh, []):
                        job()
                    if hh < H:
                        live[hh] = (proj(0, hh), proj(1, hh), proj(2, hh))
                    h = hh - lag1
                    if 0 <= h < H:
                        q, k, v = live[h]
                        live[h] = (lax.dot_general(q, k, NT, preferred_element_type=f32), v)
                    h = hh - lag2
                    if 0 <= h < H:
                        s, v = live.pop(h)
                        s = jnp.minimum(s * (scale * L2E), lim)
                        e = jnp.exp2(s - jnp.max(s, axis=-1, keepdims=True))
                        l = jnp.sum(e, axis=-1, keepdims=True)
                        rl = pl.reciprocal(l, approx=True)
                        rl = rl * (2.0 - l * rl)
                        o = jnp.dot(e.astype(bf16), v, preferred_element_type=f32) * rl
                        o_s[h * R:h * R + n, :] = o.astype(bf16)
                    for g in range(ngroups):
                        if min((g + 1) * HG - 1 + lag2 + wdel, H + lag2 - 1) == hh:
                            out_proj(g)

                out = jnp.concatenate([res[cc] for cc in range(CT)], axis=1)
                if both:
                    prev_s[...] = out[0:2 * SEG]
                    put_lhs(0, xn1)
                elif kind == 'edge2':
                    prev_s[SEG:2 * SEG, :] = out[0:SEG]
                else:
                    prev_s[0:SEG, :] = out[0:SEG]
                newm = out[n - 2 * M:]
                if kind in ('first', 'edge1'):
                    mrow = lax.broadcasted_iota(i32, (2 * M, D), 0)
                    newm = jnp.where(mrow >= M, mem0_2.astype(f32), newm)
                if xn2 is not None:
                    put_lhs(SEG, xn2)
                put_lhs(2 * SEG, newm.astype(bf16))
                if kind == 'pre':
                    @pl.when(j >= 3)
                    def _():
                        out_copy(j - 3).start()
                elif kind not in ('first', 'edge1'):
                    out_copy(j - 3).start()
                return carry
            return step

        for c in conv_copies(0):
            c.wait()
        wo_copy.wait()
        make_step('first')(0, 0)
        make_step('edge1')(1, 0)
        lax.fori_loop(2, NP, make_step('pre'), 0)
        for c in conv_copies(1):
            c.wait()
        x_copy[1].wait()
        units_step = make_step('units')
        lax.fori_loop(0, NU, lambda i, c: units_step(i + NP, c), 0)
        lax.fori_loop(NP + NU, NSEG, make_step('full'), 0)
        lax.fori_loop(NSEG, NSEG + 2, make_step('edge2'), 0)
        post(NSEG + 2, do1=False)
        out_copy(NSEG - 1).start()
        pltpu.make_async_copy(out_s, out_hbm, sems.at[3, 7]).wait()

    return kernel


def _build(S, D, H, DH, M, SEG, KS):
    NSEG, CT, NB, HP = S // SEG, D // LANES, S // BLK, H // 2
    R = 2 * SEG + 2 * M
    NU = (NB - EB) * CT // UPS
    assert DH == LANES and D % LANES == 0 and S % BLK == 0 and SEG % 16 == 0 and M % 8 == 0
    assert H % 2 == 0 and R <= LANES and KS < 8 and BLK % SEG == 0
    assert (NB - EB) * CT % UPS == 0 and EB % UPS == 0 and 2 < NP and NP + NU <= NSEG
    assert NP + CT - 1 <= EB * (BLK // SEG) and BLK // SEG > 2
    hbm = pl.BlockSpec(memory_space=pl.ANY)
    V = pltpu.VMEM
    scratch = [
        V((M, D), bf16), V((KS, D), bf16), V((D,), bf16), V((NFFT, BLK), bf16), V((BLK, NFFT), bf16),
        V((S, D), bf16),
        V((S, D), bf16),
        V((S, D), bf16),
        V((D, S), bf16),
        V((3 * HP, D, LANES), u32),
        V((3, H, D // 2, LANES), u32),
        V((H * DH, D), bf16),
        V((CT, S, LANES), f32),
        V((UPS, BLK + 16, LANES), f32),
        V((CT, 8, LANES), f32),
        V((CT * NB, XS, LANES), f32),
        V((CT * (NB + 1) + NB - 1, NFFT, LANES), f32),
        V((CT, NFFT, LANES), f32),
        V((CT, R, LANES), bf16),
        V((S + SEG, D), f32),
        V((2 * SEG, D), f32),
        V((H * R + UPS * NFFT, DH), bf16),
        V((S, D), bf16),
        V((CT, R, LANES), f32),
        V((CT, NP * SEG + 2 * M, LANES), bf16),
        V((3, H, NP * SEG + 2 * M, DH), bf16),
        pltpu.SemaphoreType.DMA((7, 16)),
    ]
    return pl.pallas_call(
        _make_kernel(S, D, H, DH, M, SEG, KS),
        out_shape=jax.ShapeDtypeStruct((S, D), bf16),
        in_specs=[hbm] * 13,
        out_specs=hbm,
        scratch_shapes=scratch,
        compiler_params=pltpu.CompilerParams(vmem_limit_bytes=120 * 1024 * 1024),
    )


@functools.partial(jax.jit, static_argnames=('A_seg_len',))
def pallas_interleave_layers__memory_aug_recurrent_mem_tr__ssm_conv_h3__prompt_kernel(
    A_x: jax.Array,
    A_mem0: jax.Array,
    A_Wq: jax.Array,
    A_Wk: jax.Array,
    A_Wv: jax.Array,
    A_Wo: jax.Array,
    A_seg_len: int,
    B_q: jax.Array,
    B_k: jax.Array,
    B_v: jax.Array,
    B_shift_k: jax.Array,
    B_ssm_k: jax.Array,
    B_ssm_D: jax.Array,
):
    del B_q
    B, S, D = A_x.shape
    H, DH = A_Wq.shape[1:]
    M = A_mem0.shape[1]
    assert B == 1
    fwd, inv = _dft_consts()
    call = _build(S, D, H, DH, M, int(A_seg_len), B_shift_k.shape[1])
    out = call(A_x.reshape(S, D), A_mem0.reshape(M, D), A_Wq, A_Wk, A_Wv, A_Wo.reshape(H * DH, D),
               B_k.reshape(S, D), B_v.reshape(S, D), B_shift_k.T, B_ssm_k, B_ssm_D, fwd, inv)
    return out.reshape(B, S, D)
```

```python
import functools

import numpy as np
import jax
import jax.numpy as jnp
from jax import lax
import jax.experimental.pallas as pl
import jax.experimental.pallas.tpu as pltpu

bf16, f32, u32, i32 = jnp.bfloat16, jnp.float32, jnp.uint32, jnp.int32

LANES = 128
BLK = 128
NFFT = 2 * BLK
L2E = 1.4426950408889634
NT = (((1,), (1,)), ((), ()))

NP = 10
EB = 4
UPS = 2
GR = 8
XO, XS = 16, NFFT + 32

PIPE = {'full': (2, 4, 8), 'units': (2, 4, 4), 'pre': (3, 6, 8), 'edge': (3, 6, 12), 'first': (0, 8, 12)}
HW = 8
HG = 2


def _dft_consts():
    f = np.arange(BLK, dtype=np.float64)[:, None] + 0.5
    m = np.arange(BLK, dtype=np.float64)[None, :]
    ang = 2.0 * np.pi * f * m / NFFT
    fwd = np.concatenate([np.cos(ang), -np.sin(ang)], axis=0)
    inv = np.concatenate([np.cos(ang).T, -np.sin(ang).T], axis=1) * (2.0 / NFFT)
    return fwd.astype(bf16), inv.astype(bf16)


def _ln(x):
    m = jnp.mean(x, axis=-1, keepdims=True)
    c = x - m
    v = jnp.mean(c * c, axis=-1, keepdims=True)
    return c * lax.rsqrt(v + 1e-5)


def _as16(words):
    return pltpu.bitcast(words, bf16)


def _ds(start, size, align):
    if isinstance(start, int):
        return pl.ds(start, size)
    return pl.ds(pl.multiple_of(start, align), size)


def _clip(j, lo, hi):
    return min(max(j, lo), hi) if isinstance(j, int) else jnp.clip(j, lo, hi)


def _make_kernel(S, D, H, DH, M, SEG, KS):
    NSEG = S // SEG
    R = 2 * SEG + 2 * M
    RE = SEG + 2 * M
    CT = D // LANES
    NB = S // BLK
    NU = (NB - EB) * CT // UPS
    GP = NB - 1
    PR = NP * SEG
    XHEAD = (NP + 2) * SEG
    ZB = H * R
    scale = DH ** -0.5

    def kernel(x_hbm, mem0_hbm, wq_hbm, wk_hbm, wv_hbm, wo_hbm, k_hbm, v_hbm, shift_hbm, ssm_hbm, ssmd_hbm,
               fwd_hbm, inv_hbm, out_hbm,
               mem0_s, shift_s, ssmd_s, fwd_s, inv_s,
               x_s, k_s, v_s, ssm_s, stage_s, pair_s, w_s, wo_s, y_s, kq_s, par_s, xg_s, gg_s, kr_s,
               lhs_s, x2_s, prev_s, o_s, out_s, acc_s, xn_s, pre_s, sems):
        w_hbm = (wq_hbm, wk_hbm, wv_hbm)
        small = [pltpu.make_async_copy(a, b, sems.at[3, 8 + i]) for i, (a, b) in enumerate(
            [(shift_hbm, shift_s), (ssmd_hbm, ssmd_s), (fwd_hbm, fwd_s), (inv_hbm, inv_s), (mem0_hbm, mem0_s)])]
        x_copy = [pltpu.make_async_copy(x_hbm.at[a:b], x_s.at[a:b], sems.at[3, i])
                  for i, (a, b) in enumerate([(0, XHEAD), (XHEAD, S)])]
        wo_copy = pltpu.make_async_copy(wo_hbm, wo_s, sems.at[3, 2])

        def conv_copies(part):
            sl = slice(0, EB * BLK) if part == 0 else slice(EB * BLK, S)
            return (pltpu.make_async_copy(k_hbm.at[sl], k_s.at[sl], sems.at[0, part]),
                    pltpu.make_async_copy(v_hbm.at[sl], v_s.at[sl], sems.at[1, part]),
                    pltpu.make_async_copy(ssm_hbm.at[:, sl], ssm_s.at[:, sl], sems.at[2, part]))

        for c in small:
            c.start()
        x_copy[0].start()
        for i in range(H // HW):
            for m in range(3):
                pltpu.make_async_copy(w_hbm[m].at[:, pl.ds(i * HW, HW), :], stage_s.at[3 * i + m],
                                      sems.at[4, 3 * i + m]).start()
        for c in conv_copies(0):
            c.start()
        wo_copy.start()
        for c in conv_copies(1):
            c.start()
        x_copy[1].start()


        for c in small:
            c.wait()
        x_copy[0].wait()
        for r0 in range(0, PR, SEG):
            xn = _ln(x_s[r0:r0 + SEG, :].astype(f32)).astype(bf16)
            for cc in range(CT):
                xn_s[cc, r0:r0 + SEG, :] = xn[:, cc * LANES:(cc + 1) * LANES]
        mem0 = mem0_s[...]
        mem0_2 = jnp.concatenate([mem0, mem0], axis=0)
        for cc in range(CT):
            xn_s[cc, PR:PR + 2 * M, :] = mem0_2[:, cc * LANES:(cc + 1) * LANES]

        def head_group(t, carry):
            m, h0 = t % 3, (t // 3) * HW
            lo_mask = jnp.full((D // 2, LANES), 0xFFFF, u32)
            pltpu.make_async_copy(stage_s.at[t], stage_s.at[t], sems.at[4, t]).wait()
            for c0 in range(0, D, 64):
                pair_s[c0 * HW // 2:(c0 + 64) * HW // 2, :] = pltpu.bitcast(
                    stage_s[t, c0:c0 + 64].reshape(64 * HW, LANES), u32)
            lhs = jnp.concatenate([xn_s[cc] for cc in range(CT)], axis=1)
            for p in range(HW // 2):
                ev = pair_s[pl.ds(p, D // 2, stride=HW), :]
                od = pair_s[pl.ds(HW // 2 + p, D // 2, stride=HW), :]
                for hh, words in enumerate(((ev & lo_mask) | (od << 16), (ev >> 16) | (od & ~lo_mask))):
                    w_s[m, h0 + 2 * p + hh] = words
                    r = jnp.dot(lhs, _as16(words), preferred_element_type=f32)
                    pre_s[m, h0 + 2 * p + hh] = r.astype(bf16)
            return carry

        lax.fori_loop(0, 3 * H // HW, head_group, 0)

        shift_t = shift_s[...].astype(f32)
        for ct in range(CT):
            cs = slice(ct * LANES, (ct + 1) * LANES)
            par_s[ct, 0:KS, :] = shift_t[:, cs]
            par_s[ct, KS:KS + 1, :] = ssmd_s[cs].astype(f32).reshape(1, LANES)

        def conv_front(a, ct, slot):
            fwd = fwd_s[...]
            cs = _ds(ct * LANES, LANES, LANES)
            r = _ds(a * BLK, BLK, BLK)
            first = isinstance(a, int) and a == 0
            if first:
                kq_s[slot, 0:16, :] = jnp.zeros((16, LANES), f32)
                kq_s[slot, 16:, :] = k_s[r, cs].astype(f32)
            else:
                kq_s[slot] = k_s[_ds(a * BLK - 16, BLK + 16, 16), cs].astype(f32)
            acc = None
            for t in range(KS):
                term = kq_s[slot, 16 - t:16 - t + BLK, :] * par_s[ct, t:t + 1, :]
                acc = term if acc is None else acc + term
            kv = (acc * v_s[r, cs].astype(f32)).astype(bf16)
            y_s[ct, r, :] = kv.astype(f32) * par_s[ct, KS:KS + 1, :]
            xg_s[ct * NB + a, XO:XO + NFFT, :] = jnp.dot(fwd, kv, preferred_element_type=f32)
            kf = lax.dot_general(fwd, ssm_s[cs, r], NT, preferred_element_type=f32)
            g = GP + ct * (NB + 1) + a
            if first:
                gg_s[g] = kf
            else:
                rows = lax.broadcasted_iota(i32, (BLK, LANES), 0)
                sgn = jnp.where((rows & 1) == 0, 1.0, -1.0).astype(f32)
                gg_s[g, 0:BLK, :] = kf[0:BLK] - sgn * kr_s[ct, BLK:NFFT, :]
                gg_s[g, BLK:NFFT, :] = kf[BLK:NFFT] + sgn * kr_s[ct, 0:BLK, :]
            kr_s[ct] = kf

        def conv_mac(a, ct, nout, zero, slot, gr):
            static = isinstance(a, int)
            g0 = GP + ct * (NB + 1) + a
            for g in range(BLK // gr):
                re = slice(g * gr, (g + 1) * gr)
                im = slice(BLK + g * gr, BLK + (g + 1) * gr)
                z = [None] * nout
                win = {}
                for b in range(a + nout if static else NB):
                    xr = xg_s[ct * NB + b, XO + re.start:XO + re.stop, :]
                    xi = xg_s[ct * NB + b, XO + im.start:XO + im.stop, :]
                    for o in range(nout):
                        c = o - b
                        if static and a + c < 0:
                            continue
                        if c not in win:
                            win[c] = (gg_s[g0 + c, re, :], gg_s[g0 + c, im, :])
                        gre, gim = win[c]
                        if z[o] is None:
                            z[o] = (gre * xr - gim * xi, gre * xi + gim * xr)
                        else:
                            z[o] = (z[o][0] + gre * xr - gim * xi, z[o][1] + gre * xi + gim * xr)
                    win.pop(nout - 1 - b, None)
                for o in range(nout):
                    zb = ZB + (slot + o) * NFFT + zero
                    o_s[_ds(zb + re.start, gr, gr), :] = z[o][0].astype(bf16)
                    o_s[_ds(zb + im.start, gr, gr), :] = z[o][1].astype(bf16)
                yield

        def conv_back(a, ct, slot):
            r = _ds(a * BLK, BLK, BLK)
            z = o_s[ZB + slot * NFFT:ZB + (slot + 1) * NFFT, :]
            y_s[ct, r, :] = y_s[ct, r, :] + jnp.dot(inv_s[...], z, preferred_element_type=f32)

        def conv_unit(a, ct, zero):
            for o in range(UPS):
                conv_front(a + o, ct, o)
                yield
            yield from conv_mac(a, ct, UPS, zero, 0, GR)
            for o in range(UPS):
                conv_back(a + o, ct, o)
            yield

        def conv_early(blocks):
            def front(a, ct, slot):
                conv_front(a, ct, slot)

            def mac(a, ct, slot):
                for _ in conv_mac(a, ct, 1, 0, slot, 16):
                    pass
            units = [(a, ct, i % UPS) for i, (a, ct) in enumerate((a, ct) for a in blocks for ct in range(CT))]
            return [functools.partial(fn, *units[t - lag])
                    for t in range(len(units) + 2) for lag, fn in enumerate((front, mac, conv_back))
                    if 0 <= t - lag < len(units)]

        def rows(seg):
            return _ds(seg * SEG, SEG, SEG)

        def load_y(seg):
            return jnp.concatenate([y_s[ct, rows(seg), :] for ct in range(CT)], axis=1)

        def put_lhs(r0, val):
            for cc in range(CT):
                lhs_s[cc, r0:r0 + val.shape[0], :] = val[:, cc * LANES:(cc + 1) * LANES]

        def out_copy(seg):
            return pltpu.make_async_copy(out_s.at[rows(seg)], out_hbm.at[rows(seg)], sems.at[3, 7])

        put_lhs(0, jnp.zeros((2 * SEG, D), bf16))
        put_lhs(2 * SEG, mem0_2)
        x2_s[0:SEG, :] = jnp.zeros((SEG, D), f32)
        prev_s[...] = jnp.zeros((2 * SEG, D), f32)

        def post(j, do1=True, do2=True):
            xn2 = None
            if do2:
                sb = _clip(j - 3, 0, NSEG - 1)
                x3 = x2_s[rows(sb), :] + prev_s[SEG:2 * SEG, :]
                out_s[rows(sb), :] = (x3 + _ln(x3) * load_y(sb)).astype(bf16)
            if do1:
                sa = _clip(j - 1, 0, NSEG - 1)
                x1 = x_s[rows(sa), :].astype(f32) + prev_s[0:SEG, :]
                x2 = x1 + _ln(x1) * load_y(sa)
                x2_s[rows(_clip(j - 1, 0, NSEG)), :] = x2
                xn2 = _ln(x2).astype(bf16)
            return xn2

        def limits(n, live):
            ri = lax.broadcasted_iota(i32, (n, n), 0)
            ci = lax.broadcasted_iota(i32, (n, n), 1)
            ntok = n - 2 * M

            def layer(i):
                if live is None:
                    return jnp.where(i < ntok, i // SEG, (i - ntok) // M)
                return jnp.where(i < ntok, 0, jnp.where((i - ntok) // M == live, 0, 1))
            ok = (layer(ri) == layer(ci)) & ((ri >= ntok) | (ci >= ntok) | (ri >= ci))
            return jnp.where(ok, 3.0e38, -1e9 * L2E).astype(f32)

        def make_step(kind):
            both = kind in ('pre', 'units', 'full')
            n = R if both else RE
            lag1, lag2, wdel = PIPE[{'edge1': 'edge', 'edge2': 'edge'}.get(kind, kind)]
            ngroups = H // HG
            if kind in ('units', 'full'):
                spans = [(0, R)]
            elif kind == 'pre':
                spans = [(SEG, R)]
            elif kind == 'edge2':
                spans = [(SEG, 2 * SEG), (2 * SEG, R)]
            else:
                spans = [(2 * SEG, R)]

            def step(j, carry):
                lim = limits(n, None if both else int(kind == 'edge2'))
                lhs = None
                if kind != 'first':
                    lhs = jnp.concatenate(
                        [jnp.concatenate([lhs_s[cc, a:b, :] for a, b in spans], axis=0)
                         for cc in range(CT)], axis=1)

                def proj(m, h):
                    if kind == 'first':
                        return jnp.concatenate([pre_s[m, h, rows(j), :], pre_s[m, h, PR:PR + 2 * M, :]], axis=0)
                    r = jnp.dot(lhs, _as16(w_s[m, h]), preferred_element_type=f32).astype(bf16)
                    if kind in ('pre', 'edge1'):
                        r = jnp.concatenate([pre_s[m, h, rows(j), :], r], axis=0)
                    return r

                side = {}
                if kind == 'units':
                    u = j - NP
                    gen = conv_unit(EB + (u // CT) * UPS, u % CT, jnp.minimum(j, 0))
                    nmac = BLK // GR
                    m0 = 2 + 2 * UPS + 3
                    at = [2 + 2 * o for o in range(UPS)]
                    at += [int(round(m0 + p * (H + lag2 - 2 - m0) / (nmac - 1))) for p in range(nmac)]
                    at.append(at[-1] + 1)
                    for hh in at:
                        side.setdefault(hh, []).append(gen.__next__)
                if kind in ('first', 'edge1'):
                    jobs = conv_early(range(0, 1) if kind == 'first' else range(1, EB))
                    for q, job in enumerate(jobs):
                        side.setdefault(q * (H + lag2) // len(jobs), []).append(job)
                if kind == 'pre':
                    nz = NB - EB
                    nx, ng = CT * nz, GP + CT * (nz + 1)
                    px, pg = -(-nx // (NP - 2)), -(-ng // (NP - 2))
                    zblk = jnp.zeros((NFFT, LANES), f32)

                    def zero_x(q):
                        kx = jnp.minimum((j - 2) * px + q, nx - 1)
                        xg_s[(kx // nz) * NB + EB + kx % nz, XO:XO + NFFT, :] = zblk

                    def zero_g(q):
                        kg = jnp.minimum((j - 2) * pg + q, ng - 1)
                        kk = jnp.maximum(kg - GP, 0)
                        gg_s[jnp.where(kg < GP, kg, GP + (kk // (nz + 1)) * (NB + 1) + EB + kk % (nz + 1))] = zblk
                    jobs = [functools.partial(zero_x, q) for q in range(px)]
                    jobs += [functools.partial(zero_g, q) for q in range(pg)]
                    for q, job in enumerate(jobs):
                        side.setdefault(q * H // len(jobs), []).append(job)

                xn2 = None if kind == 'first' else post(j, do2=(kind != 'edge1'))
                if both:
                    xn1 = _ln(x_s[rows(_clip(j + 1, 0, NSEG - 1)), :].astype(f32)).astype(bf16)

                live, res = {}, {}

                def out_proj(g):
                    ob = jnp.concatenate([o_s[h * R:h * R + n, :]
                                          for h in range(g * HG, (g + 1) * HG)], axis=1)
                    for cc in range(CT):
                        t = jnp.dot(ob, wo_s[g * HG * DH:(g + 1) * HG * DH, cc * LANES:(cc + 1) * LANES],
                                    preferred_element_type=f32)
                        if g > 0:
                            t = t + acc_s[cc, 0:n, :]
                        if g < ngroups - 1:
                            acc_s[cc, 0:n, :] = t
                        else:
                            res[cc] = t

                for hh in range(H + lag2):
                    for job in side.get(hh, []):
                        job()
                    if hh < H:
                        live[hh] = (proj(0, hh), proj(1, hh), proj(2, hh))
                    h = hh - lag1
                    if 0 <= h < H:
                        q, k, v = live[h]
                        live[h] = (lax.dot_general(q, k, NT, preferred_element_type=f32), v)
                    h = hh - lag2
                    if 0 <= h < H:
                        s, v = live.pop(h)
                        s = jnp.minimum(s * (scale * L2E), lim)
                        e = jnp.exp2(s - jnp.max(s, axis=-1, keepdims=True))
                        l = jnp.sum(e, axis=-1, keepdims=True)
                        rl = pl.reciprocal(l, approx=True)
                        rl = rl * (2.0 - l * rl)
                        o = jnp.dot(e.astype(bf16), v, preferred_element_type=f32) * rl
                        o_s[h * R:h * R + n, :] = o.astype(bf16)
                    for g in range(ngroups):
                        if min((g + 1) * HG - 1 + lag2 + wdel, H + lag2 - 1) == hh:
                            out_proj(g)

                out = jnp.concatenate([res[cc] for cc in range(CT)], axis=1)
                if both:
                    prev_s[...] = out[0:2 * SEG]
                    put_lhs(0, xn1)
                elif kind == 'edge2':
                    prev_s[SEG:2 * SEG, :] = out[0:SEG]
                else:
                    prev_s[0:SEG, :] = out[0:SEG]
                newm = out[n - 2 * M:]
                if kind in ('first', 'edge1'):
                    mrow = lax.broadcasted_iota(i32, (2 * M, D), 0)
                    newm = jnp.where(mrow >= M, mem0_2.astype(f32), newm)
                if xn2 is not None:
                    put_lhs(SEG, xn2)
                put_lhs(2 * SEG, newm.astype(bf16))
                if kind == 'pre':
                    @pl.when(j >= 3)
                    def _():
                        out_copy(j - 3).start()
                elif kind not in ('first', 'edge1'):
                    out_copy(j - 3).start()
                return carry
            return step

        for c in conv_copies(0):
            c.wait()
        wo_copy.wait()
        make_step('first')(0, 0)
        make_step('edge1')(1, 0)
        lax.fori_loop(2, NP, make_step('pre'), 0)
        for c in conv_copies(1):
            c.wait()
        x_copy[1].wait()
        units_step = make_step('units')
        lax.fori_loop(0, NU, lambda i, c: units_step(i + NP, c), 0)
        lax.fori_loop(NP + NU, NSEG, make_step('full'), 0)
        lax.fori_loop(NSEG, NSEG + 2, make_step('edge2'), 0)
        post(NSEG + 2, do1=False)
        out_copy(NSEG - 1).start()
        pltpu.make_async_copy(out_s, out_hbm, sems.at[3, 7]).wait()

    return kernel


def _build(S, D, H, DH, M, SEG, KS):
    NSEG, CT, NB = S // SEG, D // LANES, S // BLK
    R = 2 * SEG + 2 * M
    NU = (NB - EB) * CT // UPS
    assert DH == LANES and D % LANES == 0 and S % BLK == 0 and SEG % 16 == 0 and M % 8 == 0
    assert H % HW == 0 and 3 * H // HW <= 16 and R <= LANES and KS < 8 and BLK % SEG == 0
    assert (NB - EB) * CT % UPS == 0 and EB % UPS == 0 and 2 < NP and NP + NU <= NSEG
    assert NP + CT - 1 <= EB * (BLK // SEG) and BLK // SEG > 2
    hbm = pl.BlockSpec(memory_space=pl.ANY)
    V = pltpu.VMEM
    scratch = [
        V((M, D), bf16), V((KS, D), bf16), V((D,), bf16), V((NFFT, BLK), bf16), V((BLK, NFFT), bf16),
        V((S, D), bf16),
        V((S, D), bf16),
        V((S, D), bf16),
        V((D, S), bf16),
        V((3 * H // HW, D, HW, LANES), bf16),
        V((D * HW // 2, LANES), u32),
        V((3, H, D // 2, LANES), u32),
        V((H * DH, D), bf16),
        V((CT, S, LANES), f32),
        V((UPS, BLK + 16, LANES), f32),
        V((CT, 8, LANES), f32),
        V((CT * NB, XS, LANES), f32),
        V((CT * (NB + 1) + NB - 1, NFFT, LANES), f32),
        V((CT, NFFT, LANES), f32),
        V((CT, R, LANES), bf16),
        V((S + SEG, D), f32),
        V((2 * SEG, D), f32),
        V((H * R + UPS * NFFT, DH), bf16),
        V((S, D), bf16),
        V((CT, R, LANES), f32),
        V((CT, NP * SEG + 2 * M, LANES), bf16),
        V((3, H, NP * SEG + 2 * M, DH), bf16),
        pltpu.SemaphoreType.DMA((5, 16)),
    ]
    return pl.pallas_call(
        _make_kernel(S, D, H, DH, M, SEG, KS),
        out_shape=jax.ShapeDtypeStruct((S, D), bf16),
        in_specs=[hbm] * 13,
        out_specs=hbm,
        scratch_shapes=scratch,
        compiler_params=pltpu.CompilerParams(vmem_limit_bytes=120 * 1024 * 1024),
    )


@functools.partial(jax.jit, static_argnames=('A_seg_len',))
def pallas_interleave_layers__memory_aug_recurrent_mem_tr__ssm_conv_h3__prompt_kernel(
    A_x: jax.Array,
    A_mem0: jax.Array,
    A_Wq: jax.Array,
    A_Wk: jax.Array,
    A_Wv: jax.Array,
    A_Wo: jax.Array,
    A_seg_len: int,
    B_q: jax.Array,
    B_k: jax.Array,
    B_v: jax.Array,
    B_shift_k: jax.Array,
    B_ssm_k: jax.Array,
    B_ssm_D: jax.Array,
):
    del B_q
    B, S, D = A_x.shape
    H, DH = A_Wq.shape[1:]
    M = A_mem0.shape[1]
    assert B == 1
    fwd, inv = _dft_consts()
    call = _build(S, D, H, DH, M, int(A_seg_len), B_shift_k.shape[1])
    out = call(A_x.reshape(S, D), A_mem0.reshape(M, D), A_Wq, A_Wk, A_Wv, A_Wo.reshape(H * DH, D),
               B_k.reshape(S, D), B_v.reshape(S, D), B_shift_k.T, B_ssm_k, B_ssm_D, fwd, inv)
    return out.reshape(B, S, D)
```
